```python
import jax
import jax.numpy as jnp

def _softmax(x, axis=-1):
    return jax.nn.softmax(x, axis=axis)
def _gelu(x):
    return jax.nn.gelu(x, approximate=True)
def _silu(x):
    return jax.nn.silu(x)
def _sigmoid(x):
    return jax.nn.sigmoid(x)
def _layernorm(x, axis=-1, eps=1e-5):
    m = jnp.mean(x, axis=axis, keepdims=True)
    v = jnp.var(x, axis=axis, keepdims=True)
    return (x - m) / jnp.sqrt(v + eps)
def _scatter_add(tgt, idx, src, axis=0):
    return tgt.at[idx].add(src)
def _segment_sum(src, seg, n):
    return jax.ops.segment_sum(src, seg, n)
class _Rng:
    def __init__(self, key):
        self._k = key
    def _next(self):
        self._k, sub = jax.random.split(self._k)
        return sub
    def normal(self, shape):
        return jax.random.normal(self._next(), shape, dtype=jnp.bfloat16)
    def randint(self, lo, hi, shape):
        return jax.random.randint(self._next(), shape, lo, hi, dtype=jnp.int32)
    def uniform(self, shape, lo=0.0, hi=1.0):
        return jax.random.uniform(self._next(), shape, jnp.bfloat16, lo, hi)
    def permutation(self, n):
        return jax.random.permutation(self._next(), n)


kernel_name = 'concat_heads__sliding_local_dilated__compressed_kv_cla__prompt'

def setup_inputs():
    _rng = _Rng(jax.random.key(int.from_bytes(__import__("os").urandom(4), "little")))
    _w = (lambda a: (lambda t: t.astype(jnp.bfloat16) if jnp.issubdtype(t.dtype, jnp.floating) else t)(jnp.asarray(a)))
    def _A_setup():
        B, S, D = 1, 2048, 1024
        return {
            "x": _w((lambda *s: _rng.normal(s) * 0.05)(B, S, D)),
            "wqkv": _w((lambda *s: _rng.normal(s) * 0.05)(D, 3 * D)),
            "wo": _w((lambda *s: _rng.normal(s) * 0.05)(D, D)),
        }
    _A_in = _A_setup()

    def _B_setup():
        B, H, Sq, Sk, D, M = 1, 32, 2048, 2048, 128, 1024
        Dc = 4 * D
        return {
            "x": _w((lambda *s: _rng.normal(s) * 0.05)(B, Sq, M)),
            "c_kv": _w((lambda *s: _rng.normal(s) * 0.05)(B, Sk, Dc)),
            "w_q": _w((lambda *s: _rng.normal(s) * 0.05)(M, H, D) * (M ** -0.5)),
            "w_uk": _w((lambda *s: _rng.normal(s) * 0.05)(Dc, H, D) * (Dc ** -0.5)),
            "w_uv": _w((lambda *s: _rng.normal(s) * 0.05)(Dc, H, D) * (Dc ** -0.5)),
            "w_o": _w((lambda *s: _rng.normal(s) * 0.05)(H, D, M) * ((H * D) ** -0.5)),
        }
    _B_in = _B_setup()

    return {
        "A_x": _A_in["x"],
        "A_wqkv": _A_in["wqkv"],
        "A_wo": _A_in["wo"],
        "B_x": _B_in["x"],
        "B_c_kv": _B_in["c_kv"],
        "B_w_q": _B_in["w_q"],
        "B_w_uk": _B_in["w_uk"],
        "B_w_uv": _B_in["w_uv"],
        "B_w_o": _B_in["w_o"],
    }

def reference(A_x, A_wqkv, A_wo, B_x, B_c_kv, B_w_q, B_w_uk, B_w_uv, B_w_o):
    def _A_ref(x, wqkv, wo):
        B, S, D = x.shape
        H = 32; Dh = D // H
        W, dil = 8, 2
        qkv = (lambda x, *d: x.transpose(*d))((x @ wqkv).reshape(B, S, 3, H, Dh), 2, 0, 3, 1, 4)
        q, k, v = qkv[0], qkv[1], qkv[2]
        scale = Dh ** -0.5
        pos = jnp.arange(S)
        off = jnp.arange(W) * dil
        idx = pos[:, None] - off[None, :]
        mask = idx >= 0
        idx_c = jnp.where(mask, idx, 0).reshape(-1)
        kg = k[:, :, idx_c, :].reshape(B, H, S, W, Dh)
        vg = v[:, :, idx_c, :].reshape(B, H, S, W, Dh)
        logits = jnp.einsum("bhsd,bhswd->bhsw", q, kg) * scale
        logits = jnp.where(mask[None, None, :, :], logits, -1e9)
        attn = _softmax(logits, axis=-1)
        o = jnp.einsum("bhsw,bhswd->bhsd", attn, vg)
        return (lambda x, *d: x.transpose(*d))(o, 0, 2, 1, 3).reshape(B, S, D) @ wo

    def _B_ref(x, c_kv, w_q, w_uk, w_uv, w_o):
        B, Sq, M = x.shape[0], x.shape[1], x.shape[2]
        Sk = c_kv.shape[1]
        H, D = w_q.shape[1], w_q.shape[2]
        q = jnp.einsum("bqm,mhd->bhqd", x, w_q)
        k = jnp.einsum("bkc,chd->bhkd", c_kv, w_uk)
        v = jnp.einsum("bkc,chd->bhkd", c_kv, w_uv)
        scores = jnp.einsum("bhqd,bhkd->bhqk", q, k) * (D ** -0.5)
        off = Sk - Sq
        qi = jnp.arange(Sq)[:, None]
        kj = jnp.arange(Sk)[None, :]
        cmask = kj <= (qi + off)
        scores = jnp.where(cmask[None, None], scores, -1e9)
        p = _softmax(scores, axis=-1)
        ctx = jnp.einsum("bhqk,bhkd->bhqd", p, v)
        return jnp.einsum("bhqd,hdm->bqm", ctx, w_o)

    a = _A_ref(A_x, A_wqkv, A_wo)
    b = _B_ref(B_x, B_c_kv, B_w_q, B_w_uk, B_w_uv, B_w_o)
    return jnp.concatenate([a, b], axis=-1)
```

```python
import math

import jax
import jax.numpy as jnp
from jax import lax
import jax.experimental.pallas as pl
import jax.experimental.pallas.tpu as pltpu

F32, BF16, U32 = jnp.float32, jnp.bfloat16, jnp.uint32
LOG2E = math.log2(math.e)
NT_DIMS = (((1,), (1,)), ((), ()))
MASKED = -1e30

S = 2048
DM = 1024
A_DH, A_W, A_DIL = 32, 8, 2
A_HALO = 16
RA = 256
H, D, DC = 32, 128, 512
TQ = 128
RP = 512
RC = 256


def _mm(a, b):
    return jnp.dot(a, b, preferred_element_type=F32)


def _head_shuffle(chunks, lane, inverse=False):
    grp = (lane >> 2) & 7

    def rotate(x, c, left):
        if c == 0:
            return x
        if left:
            return jnp.where(grp < 8 - c, pltpu.roll(x, 128 - 4 * c, 1), pltpu.roll(x, 32 - 4 * c, 1))
        return jnp.where(grp >= c, pltpu.roll(x, 4 * c, 1), pltpu.roll(x, 128 - 32 + 4 * c, 1))

    def barrel(xs):
        xs = [xs[(-c) % 8] for c in range(8)]
        for bit in (1, 2, 4):
            sel = (grp & bit) != 0
            xs = [jnp.where(sel, xs[(c - bit) % 8], xs[c]) for c in range(8)]
        return xs

    if not inverse:
        return [rotate(x, c, True) for c, x in enumerate(barrel(chunks))]
    return barrel([rotate(x, c, False) for c, x in enumerate(chunks)])


def _shuffle_bf16(x, inverse=False):
    w = pltpu.bitcast(x, U32)
    lane = lax.broadcasted_iota(jnp.int32, (w.shape[0], 128), 1)
    out = _head_shuffle([w[:, 128 * c:128 * (c + 1)] for c in range(8)], lane, inverse)
    return pltpu.bitcast(jnp.concatenate(out, axis=1), BF16)


def _kernel(ax_hbm, wqkv_hbm, wo_hbm, bx_hbm, c_hbm, wq_hbm, wuk_hbm, wuv_hbm, wob_hbm,
            out_hbm,
            ax, wqkv, wo, bx, cc, wq_raw, wuk_raw, wuv_raw, wob,
            wq, wkv, ctx, kbuf, vbuf, obuf, in_sem, out_sem):
    loads = [pltpu.make_async_copy(src, dst, in_sem.at[i]) for i, (src, dst) in enumerate((
        (wqkv_hbm, wqkv), (ax_hbm, ax), (wo_hbm, wo),
        (wq_hbm, wq_raw), (wuk_hbm, wuk_raw), (wuv_hbm, wuv_raw),
        (bx_hbm, bx), (c_hbm, cc), (wob_hbm, wob)))]
    for cp in loads[:3]:
        cp.start()
    for cp in loads[:3]:
        cp.wait()
    for cp in loads[3:]:
        cp.start()

    def store(slot, row0, col0, rows):
        return pltpu.make_async_copy(
            obuf.at[slot], out_hbm.at[pl.ds(row0, rows), pl.ds(col0, DM)], out_sem.at[slot])

    def shuffle_w(r, _):
        rows = pl.ds(pl.multiple_of(r * 128, 128), 128)
        for part in range(3):
            cols = slice(part * DM, (part + 1) * DM)
            wqkv[rows, cols] = _shuffle_bf16(wqkv[rows, cols])

    lax.fori_loop(0, DM // 128, shuffle_w, None)
    kbuf[:, RA:, :] = jnp.zeros((8, A_HALO, 128), F32)
    vbuf[:, RA:, :] = jnp.zeros((8, A_HALO, 128), F32)

    def phase_a(t, _):
        row0 = pl.multiple_of(t * RA, RA)
        x = ax[pl.ds(row0, RA), :]
        kbuf[:, :A_HALO, :] = kbuf[:, RA:, :]
        vbuf[:, :A_HALO, :] = vbuf[:, RA:, :]
        k = _mm(x, wqkv[:, DM:2 * DM])
        for c in range(8):
            kbuf[c, A_HALO:, :] = k[:, 128 * c:128 * (c + 1)]
        q = _mm(x, wqkv[:, :DM])
        v = _mm(x, wqkv[:, 2 * DM:])
        for c in range(8):
            vbuf[c, A_HALO:, :] = v[:, 128 * c:128 * (c + 1)]

        lane = lax.broadcasted_iota(jnp.int32, (RA, 128), 1)
        pos = lax.broadcasted_iota(jnp.int32, (RA, 128), 0) + row0
        logits = []
        for w in range(A_W):
            lo = A_HALO - A_DIL * w
            acc = q[:, :128] * kbuf[0, lo:lo + RA, :]
            for c in range(1, 8):
                acc += q[:, 128 * c:128 * (c + 1)] * kbuf[c, lo:lo + RA, :]
            for bit in (1, 2):
                acc += jnp.where((lane & bit) != 0, pltpu.roll(acc, bit, 1), pltpu.roll(acc, 128 - bit, 1))
            if w > 0:
                acc = jnp.where(pos >= A_DIL * w, acc, MASKED)
            logits.append(acc)
        m = logits[0]
        for w in range(1, A_W):
            m = jnp.maximum(m, logits[w])
        p = [jnp.exp2((lg - m) * (A_DH ** -0.5 * LOG2E)) for lg in logits]
        inv = 1.0 / sum(p[1:], p[0])
        o = []
        for c in range(8):
            acc = p[0] * vbuf[c, A_HALO:, :]
            for w in range(1, A_W):
                lo = A_HALO - A_DIL * w
                acc += p[w] * vbuf[c, lo:lo + RA, :]
            o.append(acc * inv)
        o = _shuffle_bf16(jnp.concatenate(o, axis=1).astype(BF16), inverse=True)
        res = _mm(o, wo[...]).astype(BF16)

        slot = t & 1

        @pl.when(t >= 2)
        def _():
            store(slot, row0, 0, RA).wait()

        obuf[slot] = res
        store(slot, row0, 0, RA).start()

    lax.fori_loop(0, S // RA, phase_a, None)
    for slot in range(2):
        store(slot, 0, 0, RA).wait()

    for cp in loads[3:8]:
        cp.wait()

    def split_heads(raw, rows_per_step, r):
        words = raw.at[pl.ds(pl.multiple_of(r * rows_per_step * H, rows_per_step * H),
                             rows_per_step * H), :].bitcast(U32)
        for j in range(H // 2):
            even = words[pl.ds(j, rows_per_step // 2, stride=H), :]
            odd = words[pl.ds(j + H // 2, rows_per_step // 2, stride=H), :]
            yield 2 * j, pltpu.bitcast((even & jnp.uint32(0xFFFF)) | (odd << 16), BF16)
            yield 2 * j + 1, pltpu.bitcast((even >> 16) | (odd & jnp.uint32(0xFFFF0000)), BF16)

    def split_step(r, _):
        for h, val in split_heads(wq_raw, 128, r):
            wq[h, pl.ds(pl.multiple_of(r * 128, 128), 128), :] = val
        for h, val in split_heads(wuk_raw, 64, r):
            wkv[h, pl.ds(pl.multiple_of(r * 64, 64), 64), :D] = val
        for h, val in split_heads(wuv_raw, 64, r):
            wkv[h, pl.ds(pl.multiple_of(r * 64, 64), 64), D:] = val

    lax.fori_loop(0, 8, split_step, None)

    def phase_b(h, _):
        tri = (lax.broadcasted_iota(jnp.int32, (TQ, TQ), 1)
               <= lax.broadcasted_iota(jnp.int32, (TQ, TQ), 0))
        qs, ks, vs = [], [], []

        def project(i):
            rows = slice(i * RP, (i + 1) * RP)
            kv = _mm(cc[rows, :], wkv[h]).astype(BF16)
            q = (_mm(bx[rows, :], wq[h]) * (D ** -0.5 * LOG2E)).astype(BF16)
            for j in range(RP // TQ):
                tile = slice(j * TQ, (j + 1) * TQ)
                qs.append(q[tile])
                ks.append(kv[tile, :D])
                vs.append(kv[tile, D:])

        def scores(i):
            s = lax.dot_general(qs[i], jnp.concatenate(ks[:i + 1], axis=0), NT_DIMS,
                                preferred_element_type=F32)
            diag = jnp.where(tri, s[:, i * TQ:], MASKED)
            s = jnp.concatenate([s[:, :i * TQ], diag], axis=1) if i else diag
            return s, jnp.max(s, axis=1, keepdims=True)

        def context(i, s, m):
            p = jnp.exp2(s - m)
            total = jnp.sum(p, axis=1, keepdims=True)
            o = _mm(p.astype(BF16), jnp.concatenate(vs[:i + 1], axis=0))
            ctx[h, i * TQ:(i + 1) * TQ, :] = (o * (1.0 / total)).astype(BF16)

        n_tiles = S // TQ
        per = RP // TQ
        project(0)
        cur = scores(0)
        for i in range(n_tiles):
            if i % per == 0 and (i // per + 1) * RP < S:
                project(i // per + 1)
            nxt = scores(i + 1) if i + 1 < n_tiles else None
            context(i, *cur)
            cur = nxt

    lax.fori_loop(0, H, phase_b, None)

    loads[8].wait()

    def phase_c(t, _):
        row0 = pl.multiple_of(t * RC, RC)
        lhs = jnp.concatenate([ctx[h, pl.ds(row0, RC), :] for h in range(H)], axis=1)
        res = _mm(lhs, wob[...]).astype(BF16)
        slot = t & 1

        @pl.when(t >= 2)
        def _():
            store(slot, row0, DM, RC).wait()

        obuf[slot] = res
        store(slot, row0, DM, RC).start()

    lax.fori_loop(0, S // RC, phase_c, None)
    for slot in range(2):
        store(slot, 0, DM, RC).wait()


@jax.jit
def pallas_concat_heads__sliding_local_dilated__compressed_kv_cla__prompt_kernel(
    A_x: jax.Array,
    A_wqkv: jax.Array,
    A_wo: jax.Array,
    B_x: jax.Array,
    B_c_kv: jax.Array,
    B_w_q: jax.Array,
    B_w_uk: jax.Array,
    B_w_uv: jax.Array,
    B_w_o: jax.Array,
):
    assert A_x.shape == (1, S, DM) and B_x.shape == (1, S, DM) and B_c_kv.shape == (1, S, DC)
    assert B_w_q.shape == (DM, H, D) and B_w_o.shape == (H, D, DM) and RA == RC
    vmem = pltpu.VMEM
    out = pl.pallas_call(
        _kernel,
        out_shape=jax.ShapeDtypeStruct((S, 2 * DM), BF16),
        in_specs=[pl.BlockSpec(memory_space=pl.ANY)] * 9,
        out_specs=pl.BlockSpec(memory_space=pl.ANY),
        scratch_shapes=[
            vmem((S, DM), BF16), vmem((DM, 3 * DM), BF16), vmem((DM, DM), BF16),
            vmem((S, DM), BF16), vmem((S, DC), BF16),
            vmem((DM * H, D), BF16), vmem((DC * H, D), BF16), vmem((DC * H, D), BF16),
            vmem((H * D, DM), BF16),
            vmem((H, DM, D), BF16), vmem((H, DC, 2 * D), BF16), vmem((H, S, D), BF16),
            vmem((8, A_HALO + RA, 128), F32), vmem((8, A_HALO + RA, 128), F32),
            vmem((2, RA, DM), BF16),
            pltpu.SemaphoreType.DMA((9,)), pltpu.SemaphoreType.DMA((2,)),
        ],
        compiler_params=pltpu.CompilerParams(vmem_limit_bytes=110 * 1024 * 1024),
        name="concat_heads_attention",
    )(
        A_x.reshape(S, DM), A_wqkv, A_wo, B_x.reshape(S, DM), B_c_kv.reshape(S, DC),
        B_w_q.reshape(DM * H, D), B_w_uk.reshape(DC * H, D), B_w_uv.reshape(DC * H, D),
        B_w_o.reshape(H * D, DM),
    )
    return out.reshape(1, S, 2 * DM)
```

```python
import math

import jax
import jax.numpy as jnp
from jax import lax
import jax.experimental.pallas as pl
import jax.experimental.pallas.tpu as pltpu

F32, BF16, U32 = jnp.float32, jnp.bfloat16, jnp.uint32
LOG2E = math.log2(math.e)
NT_DIMS = (((1,), (1,)), ((), ()))
MASKED = -1e30

S, DM = 2048, 1024
A_DH, A_WINDOW = 32, 8
A_HALO = 16
H, D, DC = 32, 128, 512
ROWS = 256
STEPS = S // ROWS
CHUNK = 1024
TILE = 128

L_AQK, L_AV, L_AO = 1, 2, 2
L_Q, L_KV, L_O = 1, 2, 2


def _unpack(words):
    return pltpu.bitcast(words << 16, F32), pltpu.bitcast(words & jnp.uint32(0xFFFF0000), F32)


def _pack(low, high):
    return pltpu.pack_elementwise([low, high], packed_dtype=BF16)


def _chunks(x):
    return [x[:, c:c + 128] for c in range(0, x.shape[1], 128)]


_LHS = ((0, 3, 1), (2, 3, 1), (0, None, 0), (3, None, 0), (0, 1, 1), (2, 0, -1), (1, 3, -1))
_RHS = ((0, 3, 1), (0, None, 0), (1, 3, -1), (2, 0, -1), (3, None, 0), (0, 1, 1), (2, 3, 1))


def _quadrants(x):
    m, n = x.shape[0] // 2, x.shape[1] // 2
    return x[:m, :n], x[:m, n:], x[m:, :n], x[m:, n:]


def _factors(parts, words, levels, recipe):
    if levels == 0:
        return [(parts, words)]
    quads = list(zip(*[_quadrants(p) for p in parts]))
    out = []
    for a, b, sign in recipe:
        if b is None:
            out += _factors(quads[a], None if words is None else _quadrants(words)[a], levels - 1, recipe)
        else:
            mixed = [x + y if sign > 0 else x - y for x, y in zip(quads[a], quads[b])]
            out += _factors(mixed, None, levels - 1, recipe)
    return out


def _word_factors(words, levels, recipe):
    return [_pack(*parts) if plain is None else plain
            for parts, plain in _factors(_unpack(words), words, levels, recipe)]


def _strassen(lhs, rhs, levels, marks=None, base=0):
    if levels == 0:
        out = jnp.dot(pltpu.bitcast(lhs(base), BF16), pltpu.bitcast(rhs(base), BF16),
                      preferred_element_type=F32)
        if marks is not None:
            marks(out)
        return out
    step = 7 ** (levels - 1)
    m3, m4, m5, m2, m1, m6, m7 = [_strassen(lhs, rhs, levels - 1, marks, base + i * step)
                                  for i in (2, 3, 4, 1, 0, 5, 6)]
    return jnp.concatenate([jnp.concatenate([m4 - m5 + m1 + m7, m3 + m5], axis=1),
                            jnp.concatenate([m2 + m4, m3 - m2 + m1 + m6], axis=1)], axis=0)


def _factor_shape(rows, cols, levels):
    return (7 ** levels, rows >> levels, cols >> levels)


def _slab(load, total, levels, start, n):
    return jnp.concatenate([load((total >> levels) * b + start, n) for b in range(2 ** levels)], axis=0)


def _keep(step):
    return lax.broadcasted_iota(jnp.int32, (8, 128), 1) + step >= 0


def _after(x, token, keep):
    return jnp.where(keep, x, pltpu.bitcast(token, x.dtype))


def _collect(tokens, row_step, col_step):
    return lambda prod: tokens.extend(prod[r:r + 8, c:c + 128] for c in range(0, prod.shape[1], col_step)
                                      for r in range(0, prod.shape[0], row_step))


def _store_spread(jobs, tokens, keep):
    total = sum(words.size for _, words in jobs) // 1024
    n = 0
    for store, words in jobs:
        rows = []
        for r in range(0, words.shape[0], 8):
            cols = []
            for piece in _chunks(words[r:r + 8]):
                cols.append(_after(piece, tokens[n * len(tokens) // total], keep))
                n += 1
            rows.append(jnp.concatenate(cols, axis=1))
        store(jnp.concatenate(rows, axis=0))


def _head_shuffle(chunks, inverse=False):
    group = (lax.broadcasted_iota(jnp.int32, chunks[0].shape, 1) >> 2) & 7

    def rotate(x, c):
        if c == 0:
            return x
        if inverse:
            return jnp.where(group >= c, pltpu.roll(x, 4 * c, 1), pltpu.roll(x, 96 + 4 * c, 1))
        return jnp.where(group < 8 - c, pltpu.roll(x, 128 - 4 * c, 1), pltpu.roll(x, 32 - 4 * c, 1))

    def exchange(xs):
        xs = [xs[-c % 8] for c in range(8)]
        for bit in (1, 2, 4):
            xs = [jnp.where((group & bit) != 0, xs[(c - bit) % 8], xs[c]) for c in range(8)]
        return xs

    if inverse:
        return jnp.concatenate(exchange([rotate(x, c) for c, x in enumerate(chunks)]), axis=1)
    return jnp.concatenate([rotate(x, c) for c, x in enumerate(exchange(chunks))], axis=1)


def _attention_order(n_tiles, lead=8, hold=3):
    tiles = [(e, i) for i in reversed(range(n_tiles)) for e in range(2)]
    steps, done = [], 0
    for t, tile in enumerate(tiles):
        steps.append(("scores", tile))
        while sum(i + 1 for _, i in tiles[done + 1:t + 1]) >= lead:
            steps.append(("context", tiles[done]))
            if done >= hold:
                steps.append(("store", tiles[done - hold]))
            done += 1
    steps += [("context", tile) for tile in tiles[done:]]
    steps += [("store", tile) for tile in tiles[done - hold:]]
    return steps


def _kernel(ax_hbm, wqkv_hbm, wo_hbm, bx_hbm, c_hbm, wq_hbm, wuk_hbm, wuv_hbm, wob_hbm, out_hbm,
            wq_raw, wuk_raw, wuv_raw, wob, x_fac, c_fac, wq_fac, wkv_fac, wo_fac, qkv, in_sem, out_sem):
    head_loads = [pltpu.make_async_copy(src.bitcast(U32).at[:, pl.ds(8 * g, 8), :], dst.at[g], in_sem.at[0])
                  for g in range(2) for src, dst in ((wq_hbm, wq_raw), (wuk_hbm, wuk_raw), (wuv_hbm, wuv_raw))]
    wob_load = pltpu.make_async_copy(wob_hbm.bitcast(U32), wob, in_sem.at[1])

    def pair_factors(j, kv_starts, q_starts):
        def head_rows(raw, start, n):
            rows = raw.shape[1]
            first = ((j >> 3) * rows + start) * 8 + (j & 7)
            return _unpack(raw.reshape(2 * rows * 8, D)[pl.ds(first, n, stride=8), :])

        for raws, fac, total, levels, starts in (((wuk_raw, wuv_raw), wkv_fac, DC, L_KV, kv_starts),
                                                 ((wq_raw,), wq_fac, DM, L_Q, q_starts)):
            def load(start, n, raws=raws):
                return jnp.concatenate([y for raw in raws for y in head_rows(raw, start, n)], axis=1)

            for start in starts:
                for i, ((y,), _) in enumerate(_factors([_slab(load, total, levels, start, 16)], None, levels, _RHS)):
                    def store(val, fac=fac, i=i, start=start):
                        fac[i, pl.ds(start, 16), :] = val.astype(BF16)
                    yield store, y

    def project_a(ax, w_raw, bx, cc, q_fac, k_fac, v_fac, sem):
        slab = DM // 8 // STEPS

        def weight_copy(part, t):
            rows = pl.ds(t * slab, slab)
            return pltpu.make_async_copy(wqkv_hbm.bitcast(U32).at[:, rows, pl.ds(part * DM, DM)],
                                         w_raw.at[part, :, rows, :], sem.at[part * STEPS + t])

        def x_copy(t):
            rows = pl.ds(t * (ROWS // 2), ROWS // 2)
            return pltpu.make_async_copy(ax_hbm.bitcast(U32).at[rows], ax.at[rows], sem.at[3 * STEPS + t])

        later_loads = [pltpu.make_async_copy(src.bitcast(U32), dst, sem.at[4 * STEPS + i])
                       for i, (src, dst) in enumerate(((wo_hbm, w_raw.at[3]), (bx_hbm, bx), (c_hbm, cc)))]
        for t in range(STEPS):
            weight_copy(1, t).start()
        for t in range(STEPS):
            for copy in (x_copy(t), weight_copy(0, t), weight_copy(2, t)):
                copy.start()
        for copy in later_loads + head_loads + [wob_load]:
            copy.start()

        def weight_factors(part, fac, levels, t):
            start = pl.multiple_of(t * slab, slab)
            quarters = [w_raw[part, b, pl.ds(start, slab), :] for b in range(4)]
            if part < 3:
                quarters = [_head_shuffle(_chunks(w)) for w in quarters]
            for e in range(4 >> levels):
                words = jnp.concatenate(quarters[e::4 >> levels], axis=0)
                for i, y in enumerate(_word_factors(words, levels, _RHS)):
                    def store(val, i=i, e=e):
                        fac[i, pl.ds(start + e * (DM // 8), slab), :] = val
                    yield store, y

        def prepare_keys(t, _):
            weight_copy(1, t).wait()
            for store, words in weight_factors(1, k_fac, L_AQK, t):
                store(words)

        lax.fori_loop(0, STEPS, prepare_keys, None)
        qkv[1:, :, :A_HALO, :] = jnp.zeros((2, 8, A_HALO, 128), BF16)

        def project(part, fac, levels, t, tokens):
            x = ax[pl.ds(pl.multiple_of(t * (ROWS // 2), ROWS // 2), ROWS // 2), :]
            lhs = _word_factors(x, levels, _LHS)
            out = _strassen(lambda i: lhs[i], lambda i: fac[i], levels, _collect(tokens, 8, 256))
            if part == 0:
                out = out * (A_DH ** -0.5 * LOG2E)
            for c, y in enumerate(_chunks(out)):
                qkv[part, c, pl.ds(pl.multiple_of(t * ROWS + A_HALO, A_HALO), ROWS), :] = y.astype(BF16)

        def keys(t, _):
            for copy in (x_copy(t), weight_copy(0, t), weight_copy(2, t)):
                copy.wait()
            tokens = []
            project(1, k_fac, L_AQK, t, tokens)
            _store_spread([*weight_factors(0, q_fac, L_AQK, t), *weight_factors(2, v_fac, L_AV, t)],
                          tokens, _keep(t))

        lax.fori_loop(0, STEPS, keys, None)
        for copy in later_loads:
            copy.wait()

        def queries_values(t, _):
            tokens = []
            project(0, q_fac, L_AQK, t, tokens)
            project(2, v_fac, L_AV, t, tokens)
            jobs = list(weight_factors(3, wo_fac, L_AO, t))
            for src, fac, levels in ((bx, x_fac, L_Q), (cc, c_fac, L_KV)):
                per_chunk = STEPS // (S // CHUNK)
                n = (CHUNK // 2 >> levels) // per_chunk
                chunk, start = t // per_chunk, pl.multiple_of((t % per_chunk) * n, n)

                def load(row, m, src=src, chunk=chunk):
                    return src[pl.ds(pl.multiple_of(chunk * (CHUNK // 2) + row, m), m), :]

                for i, y in enumerate(_word_factors(_slab(load, CHUNK // 2, levels, start, n), levels, _LHS)):
                    def store(val, fac=fac, chunk=chunk, i=i, start=start, n=n):
                        fac[chunk, i, pl.ds(start, n), :] = val
                    jobs.append((store, y))
            _store_spread(jobs, tokens, _keep(t))

        lax.fori_loop(0, STEPS, queries_values, None)
        for copy in head_loads:
            copy.wait()

        def first_pair(t, _):
            start = pl.multiple_of(t * 16, 16)
            for store, val in pair_factors(0, [start], [start + 128 * a for a in range(4)]):
                store(val)

        lax.fori_loop(0, 8, first_pair, None)

    pl.run_scoped(
        project_a,
        pltpu.VMEM((S // 2, DM), U32), pltpu.VMEM((4, 4, DM // 8, DM), U32),
        pltpu.VMEM((S // 2, DM), U32), pltpu.VMEM((S // 2, DC), U32),
        pltpu.VMEM(_factor_shape(DM // 2, DM, L_AQK), U32), pltpu.VMEM(_factor_shape(DM // 2, DM, L_AQK), U32),
        pltpu.VMEM(_factor_shape(DM // 2, DM, L_AV), U32), pltpu.SemaphoreType.DMA((4 * STEPS + 3,)))

    def attend(ctx, wob_fac, result, kv32):
        wob_load.wait()

        def head_pair(j, _):
            below = (lax.broadcasted_iota(jnp.int32, (TILE, TILE), 1)
                     <= lax.broadcasted_iota(jnp.int32, (TILE, TILE), 0))
            keep = _keep(j)
            qs, ks, vs, scores, results, stored = {}, {}, {}, {}, {}, []

            following = list(pair_factors(jnp.minimum(j + 1, H // 2 - 1),
                                          range(0, DC >> L_KV, 16), range(0, DM >> L_Q, 16)))
            n_kv = 7 ** L_KV * (DC >> L_KV) // 16
            jobs = following[:n_kv]
            per_pair = (H * D // 2 >> L_O) // (H // 2)
            for start in range(0, per_pair, 8):
                start = pl.multiple_of(j * per_pair + start, 8)
                words = _slab(lambda row, n: wob[pl.ds(pl.multiple_of(row, n), n), :], H * D // 2, L_O, start, 8)
                for i, y in enumerate(_word_factors(words, L_O, _RHS)):
                    def store(val, i=i, start=start):
                        wob_fac[i, pl.ds(start, 8), :] = val
                    jobs.append((store, y))

            def run_jobs(prod):
                for r in range(0, prod.shape[0], 8):
                    if jobs:
                        store, val = jobs.pop(0)
                        head = jnp.concatenate([_after(y, prod[r:r + 8], keep) for y in _chunks(val[:8])], axis=1)
                        store(jnp.concatenate([head, val[8:]], axis=0) if val.shape[0] > 8 else head)

            for chunk in range(S // CHUNK):
                kv = _strassen(lambda i: c_fac[chunk, i], lambda i: wkv_fac.bitcast(U32)[i], L_KV).astype(BF16)
                for t in range(CHUNK // TILE):
                    k0, k1, v0, v1 = _chunks(kv[t * TILE:(t + 1) * TILE])
                    i = chunk * (CHUNK // TILE) + t
                    ks[0, i], ks[1, i], vs[0, i], vs[1, i] = k0, k1, v0, v1
            for chunk in range(S // CHUNK):
                q = _strassen(lambda i: x_fac[chunk, i], lambda i: wq_fac.bitcast(U32)[i], L_Q, run_jobs)
                q = q * (D ** -0.5 * LOG2E)
                for t in range(CHUNK // TILE):
                    i = chunk * (CHUNK // TILE) + t
                    qs[0, i], qs[1, i] = _chunks(q[t * TILE:(t + 1) * TILE])
            assert not jobs
            for store, val in following[n_kv:]:
                store(val)

            def score(e, i):
                q = qs[e, i]
                while stored:
                    e0, i0 = stored.pop()
                    token = ctx.bitcast(U32)[2 * j + e0 + (j >> 8), i0 * TILE // 2:i0 * TILE // 2 + 8, :]
                    q = jnp.concatenate([_after(q[:8], token, keep), q[8:]], axis=0)
                s = lax.dot_general(q.astype(BF16), jnp.concatenate([ks[e, t] for t in range(i + 1)], axis=0),
                                    NT_DIMS, preferred_element_type=F32)
                diagonal = jnp.where(below, s[:, i * TILE:], MASKED)
                s = jnp.concatenate([s[:, :i * TILE], diagonal], axis=1) if i else diagonal
                scores[e, i] = s, jnp.max(s, axis=1, keepdims=True)

            def context(e, i):
                s, top = scores.pop((e, i))
                p = jnp.exp2(s - top)
                total = jnp.sum(p, axis=1, keepdims=True)
                o = jnp.dot(p.astype(BF16), jnp.concatenate([vs[e, t] for t in range(i + 1)], axis=0),
                            preferred_element_type=F32)
                inv = pl.reciprocal(total, approx=True)
                results[e, i] = (o * (inv * (2.0 - total * inv))).astype(BF16)

            def store_tile(e, i):
                ctx[2 * j + e, i * TILE:(i + 1) * TILE, :] = results.pop((e, i))
                stored.append((e, i))

            for name, tile in _attention_order(S // TILE):
                {"scores": score, "context": context, "store": store_tile}[name](*tile)

        lax.fori_loop(0, H // 2, head_pair, None)

        def out_copy(t):
            return pltpu.make_async_copy(result.at[t & 1], out_hbm.at[pl.ds(pl.multiple_of(t * ROWS, ROWS), ROWS)],
                                         out_sem.at[t & 1])

        def window_attention(t, tokens):
            half, halo = ROWS // 2, A_HALO // 2
            first = pl.multiple_of(t * half, half)
            for part in (1, 2):
                for c in range(8):
                    for e, y in enumerate(_unpack(qkv.bitcast(U32)[part, c, pl.ds(first, halo + half), :])):
                        kv32[part - 1, e, c] = y
            lane = lax.broadcasted_iota(jnp.int32, (8, 128), 1)
            position = lax.broadcasted_iota(jnp.int32, (8, 128), 0) + first
            keep = _keep(t)
            period = (len(tokens) - 42) / (ROWS // 8)

            def at(y, when):
                return _after(y, tokens[min(int(when), len(tokens) - 1)], keep)

            out = []
            for r in range(0, half, 8):
                both = []
                for e, q in enumerate(zip(*[_unpack(qkv.bitcast(U32)[0, c, pl.ds(first + halo + r, 8), :])
                                            for c in range(8)])):
                    t0 = (r // 4 + e) * period
                    logits = []
                    for w in range(A_WINDOW):
                        terms = [q[c] * kv32[0, e, c, halo + r - w:halo + r - w + 8, :] for c in range(8)]
                        logits.append(at(sum(terms[1:], terms[0]), t0 + w))
                    for bit, lag in ((1, 4), (2, 8)):
                        logits = [at(y + jnp.where((lane & bit) != 0, pltpu.roll(y, bit, 1),
                                                   pltpu.roll(y, 128 - bit, 1)), t0 + lag + w)
                                  for w, y in enumerate(logits)]
                    logits = [jnp.where(position + r >= w, y, MASKED) if r < w else y
                              for w, y in enumerate(logits)]
                    top = logits[0]
                    for y in logits[1:]:
                        top = jnp.maximum(top, y)
                    p = [jnp.exp2(y - top) for y in logits]
                    total = sum(p[1:], p[0])
                    inv = pl.reciprocal(total, approx=True)
                    inv = at(inv * (2.0 - total * inv), t0 + 17)
                    p = [y * inv for y in p]
                    o = []
                    for c in range(8):
                        terms = [p[w] * kv32[1, e, c, halo + r - w:halo + r - w + 8, :] for w in range(A_WINDOW)]
                        o.append(at(sum(terms[1:], terms[0]), t0 + 19 + c))
                    both.append(o)
                words = _head_shuffle([_pack(even, odd) for even, odd in zip(*both)], inverse=True)
                out.append(jnp.concatenate([at(y, r // 4 * period + 34 + c) for c, y in enumerate(_chunks(words))],
                                           axis=1))
            return jnp.concatenate(out, axis=0)

        def outputs(t, _):
            @pl.when(t >= 2)
            def _():
                out_copy(t - 2).wait()

            tokens = []
            rows = pl.ds(pl.multiple_of(t * (ROWS // 2), ROWS // 2), ROWS // 2)
            lhs_b = _word_factors(jnp.concatenate([ctx.bitcast(U32)[h, rows, :] for h in range(H)], axis=1),
                                  L_O, _LHS)
            result[t & 1, :, DM:] = _strassen(lambda i: lhs_b[i], lambda i: wob_fac[i], L_O,
                                              _collect(tokens, 16, 128)).astype(BF16)
            lhs_a = _word_factors(window_attention(t, tokens), L_AO, _LHS)
            result[t & 1, :, :DM] = _strassen(lambda i: lhs_a[i], lambda i: wo_fac[i], L_AO).astype(BF16)
            out_copy(t).start()

        lax.fori_loop(0, STEPS, outputs, None)
        for t in (STEPS - 2, STEPS - 1):
            out_copy(t).wait()

    pl.run_scoped(
        attend,
        pltpu.VMEM((H, S, D), BF16), pltpu.VMEM(_factor_shape(H * D // 2, DM, L_O), U32),
        pltpu.VMEM((2, ROWS, 2 * DM), BF16), pltpu.VMEM((2, 2, 8, (A_HALO + ROWS) // 2, 128), F32))


@jax.jit
def pallas_concat_heads__sliding_local_dilated__compressed_kv_cla__prompt_kernel(
    A_x: jax.Array,
    A_wqkv: jax.Array,
    A_wo: jax.Array,
    B_x: jax.Array,
    B_c_kv: jax.Array,
    B_w_q: jax.Array,
    B_w_uk: jax.Array,
    B_w_uv: jax.Array,
    B_w_o: jax.Array,
):
    assert A_x.shape == B_x.shape == (1, S, DM) and B_c_kv.shape == (1, S, DC)
    assert B_w_q.shape == (DM, H, D) and B_w_uk.shape == B_w_uv.shape == (DC, H, D)
    out = pl.pallas_call(
        _kernel,
        out_shape=jax.ShapeDtypeStruct((S, 2 * DM), BF16),
        in_specs=[pl.BlockSpec(memory_space=pl.ANY)] * 9,
        out_specs=pl.BlockSpec(memory_space=pl.ANY),
        scratch_shapes=[
            pltpu.VMEM((2, DM, 8, D), U32), pltpu.VMEM((2, DC, 8, D), U32), pltpu.VMEM((2, DC, 8, D), U32),
            pltpu.VMEM((H * D // 2, DM), U32),
            pltpu.VMEM((S // CHUNK,) + _factor_shape(CHUNK // 2, DM, L_Q), U32),
            pltpu.VMEM((S // CHUNK,) + _factor_shape(CHUNK // 2, DC, L_KV), U32),
            pltpu.VMEM(_factor_shape(DM, 2 * D, L_Q), BF16), pltpu.VMEM(_factor_shape(DC, 4 * D, L_KV), BF16),
            pltpu.VMEM(_factor_shape(DM // 2, DM, L_AO), U32), pltpu.VMEM((3, 8, A_HALO + S, 128), BF16),
            pltpu.SemaphoreType.DMA((2,)), pltpu.SemaphoreType.DMA((2,)),
        ],
        compiler_params=pltpu.CompilerParams(vmem_limit_bytes=120 * 1024 * 1024),
        name="concat_heads_attention",
    )(
        A_x.reshape(S, DM), A_wqkv.reshape(4, DM // 4, 3 * DM), A_wo.reshape(4, DM // 4, DM),
        B_x.reshape(S, DM), B_c_kv.reshape(S, DC),
        B_w_q, B_w_uk, B_w_uv, B_w_o.reshape(H * D, DM),
    )
    return out.reshape(1, S, 2 * DM)
```

```python
import math

import jax
import jax.numpy as jnp
from jax import lax
import jax.experimental.pallas as pl
import jax.experimental.pallas.tpu as pltpu

F32, BF16, U32 = jnp.float32, jnp.bfloat16, jnp.uint32
LOG2E = math.log2(math.e)
NT_DIMS = (((1,), (1,)), ((), ()))
MASKED = -1e30

S, DM = 2048, 1024
A_DH, A_WINDOW = 32, 8
A_HALO = 16
H, D, DC = 32, 128, 512
ROWS = 256
STEPS = S // ROWS
CHUNK = 1024
TILE = 128
LEVELS = 2
PRODUCTS = 7 ** LEVELS


def _unpack(words):
    return pltpu.bitcast(words << 16, F32), pltpu.bitcast(words & jnp.uint32(0xFFFF0000), F32)


def _pack(low, high):
    return pltpu.pack_elementwise([low, high], packed_dtype=BF16)


def _chunks(x):
    return [x[:, c:c + 128] for c in range(0, x.shape[1], 128)]


_LHS = ((0, 3, 1), (2, 3, 1), (0, None, 0), (3, None, 0), (0, 1, 1), (2, 0, -1), (1, 3, -1))
_RHS = ((0, 3, 1), (0, None, 0), (1, 3, -1), (2, 0, -1), (3, None, 0), (0, 1, 1), (2, 3, 1))


def _quadrants(x):
    m, n = x.shape[0] // 2, x.shape[1] // 2
    return x[:m, :n], x[:m, n:], x[m:, :n], x[m:, n:]


def _factors(parts, words, levels, recipe):
    if levels == 0:
        return [(parts, words)]
    quads = list(zip(*[_quadrants(p) for p in parts]))
    out = []
    for a, b, sign in recipe:
        if b is None:
            out += _factors(quads[a], None if words is None else _quadrants(words)[a], levels - 1, recipe)
        else:
            mixed = [x + y if sign > 0 else x - y for x, y in zip(quads[a], quads[b])]
            out += _factors(mixed, None, levels - 1, recipe)
    return out


def _word_factors(words, recipe):
    return [_pack(*parts) if plain is None else plain
            for parts, plain in _factors(_unpack(words), words, LEVELS, recipe)]


def _f32_factors(x, recipe):
    return [y for (y,), _ in _factors([x], None, LEVELS, recipe)]


def _dot(a, b):
    a, b = [y if y.dtype == BF16 else pltpu.bitcast(y, BF16) for y in (a, b)]
    return jnp.dot(a, b, preferred_element_type=F32)


def _strassen(lhs, rhs, watch=None, levels=LEVELS, base=0):
    if levels == 0:
        out = _dot(lhs(base), rhs(base))
        if watch is not None:
            watch(out)
        return out
    step = 7 ** (levels - 1)
    m3, m4, m5, m2, m1, m6, m7 = [_strassen(lhs, rhs, watch, levels - 1, base + i * step)
                                  for i in (2, 3, 4, 1, 0, 5, 6)]
    return jnp.concatenate([jnp.concatenate([m4 - m5 + m1 + m7, m3 + m5], axis=1),
                            jnp.concatenate([m2 + m4, m3 - m2 + m1 + m6], axis=1)], axis=0)


def _slab(load, total, start, n):
    return jnp.concatenate([load(total // 4 * b + start, n) for b in range(4)], axis=0)


def _keep(step):
    return lax.broadcasted_iota(jnp.int32, (8, 128), 1) + step >= 0


def _after(x, token, keep):
    return jnp.where(keep, x, pltpu.bitcast(token, x.dtype))


def _collect(tokens, row_step, col_step):
    return lambda prod: tokens.extend(prod[r:r + 8, c:c + 128] for c in range(0, prod.shape[1], col_step)
                                      for r in range(0, prod.shape[0], row_step))


def _store_spread(jobs, tokens, keep):
    def height(val):
        return 8 if val.dtype == U32 else 16

    total = sum(val.size // (128 * height(val)) for _, val in jobs)
    n = 0
    for store, val in jobs:
        rows = []
        for r in range(0, val.shape[0], height(val)):
            cols = []
            for piece in _chunks(val[r:r + 8]):
                cols.append(_after(piece, tokens[n * len(tokens) // total], keep))
                n += 1
            rows.append(jnp.concatenate(cols, axis=1))
            if height(val) == 16:
                rows.append(val[r + 8:r + 16])
        store(jnp.concatenate(rows, axis=0))


def _head_shuffle(chunks, inverse=False):
    group = (lax.broadcasted_iota(jnp.int32, chunks[0].shape, 1) >> 2) & 7

    def rotate(x, c):
        if c == 0:
            return x
        if inverse:
            return jnp.where(group >= c, pltpu.roll(x, 4 * c, 1), pltpu.roll(x, 96 + 4 * c, 1))
        return jnp.where(group < 8 - c, pltpu.roll(x, 128 - 4 * c, 1), pltpu.roll(x, 32 - 4 * c, 1))

    def exchange(xs):
        xs = [xs[-c % 8] for c in range(8)]
        for bit in (1, 2, 4):
            xs = [jnp.where((group & bit) != 0, xs[(c - bit) % 8], xs[c]) for c in range(8)]
        return xs

    if inverse:
        return jnp.concatenate(exchange([rotate(x, c) for c, x in enumerate(chunks)]), axis=1)
    return jnp.concatenate([rotate(x, c) for c, x in enumerate(exchange(chunks))], axis=1)


def _attention_order(n_tiles, lead=8, hold=3):
    tiles = [(e, i) for i in reversed(range(n_tiles)) for e in range(2)]
    steps, done = [], 0
    for t, tile in enumerate(tiles):
        steps.append(("scores", tile))
        while sum(i + 1 for _, i in tiles[done + 1:t + 1]) >= lead:
            steps.append(("context", tiles[done]))
            if done >= hold:
                steps.append(("store", tiles[done - hold]))
            done += 1
    steps += [("context", tile) for tile in tiles[done:]]
    steps += [("store", tile) for tile in tiles[done - hold:]]
    return steps


def _sum(terms):
    return sum(terms[1:], terms[0])


def _kernel(ax_hbm, wqkv_hbm, wo_hbm, bx_hbm, c_hbm, wq_hbm, wuk_hbm, wuv_hbm, wob_hbm, out_hbm,
            wuk_raw, wuv_raw, c_fac, wkv_fac, wo_fac, ctx, mixed, in_sem, out_sem):
    kv_loads = [pltpu.make_async_copy(src.bitcast(U32).at[:, pl.ds(8 * g, 8), :], dst.at[g], in_sem)
                for g in range(2) for src, dst in ((wuk_hbm, wuk_raw), (wuv_hbm, wuv_raw))]

    def head_rows(raw, j, start, n):
        rows = math.prod(raw.shape[1:-2])
        first = ((j >> 3) * rows + start) * 8 + (j & 7)
        return _unpack(raw.reshape(2 * rows * 8, D)[pl.ds(first, n, stride=8), :])

    def kv_factors(j, starts):
        def load(start, n):
            return jnp.concatenate([y for raw in (wuk_raw, wuv_raw) for y in head_rows(raw, j, start, n)], axis=1)

        for start in starts:
            for i, y in enumerate(_f32_factors(_slab(load, DC, start, 16), _RHS)):
                def store(val, i=i, start=start):
                    wkv_fac[i, pl.ds(start, 16), :] = val.astype(BF16)
                yield store, y

    def word_rows(t):
        return pl.ds(pl.multiple_of(t * (ROWS // 2), ROWS // 2), ROWS // 2)

    def project(bx, qkv, wq_fac, bx_sem):
        bx_load = pltpu.make_async_copy(bx_hbm.bitcast(U32), bx, bx_sem)

        def project_a(ax, w_raw, cc, q_w, k_w, v_fac, wq_raw, sem):
            slab = DM // 8 // STEPS

            def weight_copy(part, t):
                rows = pl.ds(t * slab, slab)
                return pltpu.make_async_copy(wqkv_hbm.bitcast(U32).at[:, rows, pl.ds(part * DM, DM)],
                                             w_raw.at[part, :, rows, :], sem.at[part * STEPS + t])

            def x_copy(t):
                rows = pl.ds(t * (ROWS // 2), ROWS // 2)
                return pltpu.make_async_copy(ax_hbm.bitcast(U32).at[rows], ax.at[rows], sem.at[3 * STEPS + t])

            def wq_copies(t):
                rows = pl.ds(t * 2 * slab, 2 * slab)
                return [pltpu.make_async_copy(wq_hbm.bitcast(U32).at[:, rows, pl.ds(8 * g, 8), :],
                                              wq_raw.at[g, :, rows], sem.at[4 * STEPS + t]) for g in range(2)]

            later_loads = [pltpu.make_async_copy(src.bitcast(U32), dst, sem.at[5 * STEPS + i])
                           for i, (src, dst) in enumerate(((wo_hbm, w_raw.at[3]), (c_hbm, cc)))]
            for t in range(STEPS):
                weight_copy(1, t).start()
            for t in range(STEPS):
                for copy in (x_copy(t), weight_copy(0, t), weight_copy(2, t)):
                    copy.start()
            for copy in later_loads:
                copy.start()

            def weights(part, t):
                rows = pl.ds(pl.multiple_of(t * slab, slab), slab)
                quarters = [w_raw[part, b, rows, :] for b in range(4)]
                if part < 3:
                    quarters = [_head_shuffle(_chunks(w)) for w in quarters]
                if part >= 2:
                    quarters = _word_factors(jnp.concatenate(quarters, axis=0), _RHS)
                for i, y in enumerate(quarters):
                    def store(val, i=i):
                        (q_w, k_w, v_fac, wo_fac)[part][i, rows, :] = val
                    yield store, y

            def prepare_keys(t, _):
                weight_copy(1, t).wait()
                for store, words in weights(1, t):
                    store(words)

            lax.fori_loop(0, STEPS, prepare_keys, None)
            for t in range(STEPS):
                for copy in wq_copies(t):
                    copy.start()
            for copy in [bx_load] + kv_loads:
                copy.start()
            qkv[1:, :, :A_HALO, :] = jnp.zeros((2, 8, A_HALO, 128), BF16)

            def project_rows(part, t, tokens):
                x = ax[word_rows(t), :]
                if part < 2:
                    out = _dot(x, jnp.concatenate([(q_w, k_w)[part][b] for b in range(4)], axis=0))
                    _collect(tokens, 8, 128)(out)
                else:
                    lhs = _word_factors(x, _LHS)
                    out = _strassen(lambda i: lhs[i], lambda i: v_fac[i], _collect(tokens, 32, 256))
                if part == 0:
                    out = out * (A_DH ** -0.5 * LOG2E)
                for c, y in enumerate(_chunks(out)):
                    qkv[part, c, pl.ds(pl.multiple_of(t * ROWS + A_HALO, A_HALO), ROWS), :] = y.astype(BF16)

            def keys(t, _):
                for copy in (x_copy(t), weight_copy(0, t), weight_copy(2, t)):
                    copy.wait()
                tokens = []
                project_rows(1, t, tokens)
                _store_spread([*weights(0, t), *weights(2, t)], tokens, _keep(t))

            lax.fori_loop(0, STEPS, keys, None)
            for copy in later_loads:
                copy.wait()

            def queries_values(t, _):
                for copy in wq_copies(t):
                    copy.wait()
                tokens = []
                project_rows(0, t, tokens)
                project_rows(2, t, tokens)
                jobs = list(weights(3, t))
                per_chunk = STEPS // (S // CHUNK)
                n = CHUNK // 8 // per_chunk
                chunk, start = t // per_chunk, pl.multiple_of((t % per_chunk) * n, n)
                words = _slab(lambda row, m: cc[pl.ds(pl.multiple_of(chunk * (CHUNK // 2) + row, m), m), :],
                              CHUNK // 2, start, n)
                for i, y in enumerate(_word_factors(words, _LHS)):
                    def store(val, i=i):
                        c_fac[chunk, i, pl.ds(start, n), :] = val
                    jobs.append((store, y))
                for piece in range(0, 2 * slab, 16):
                    first = pl.multiple_of(t * 2 * slab + piece, 16)
                    for pair in range(4):
                        def load(row, m):
                            return jnp.concatenate([y for quarter in range(4)
                                                    for y in head_rows(wq_raw, 4 * quarter + pair, row, m)], axis=1)

                        for i, y in enumerate(_f32_factors(_slab(load, DM, first, 16), _RHS)):
                            for e, head in enumerate(_chunks(y)):
                                def store(val, i=i, slot=2 * pair + e, first=first):
                                    wq_fac[i, slot, pl.ds(first, 16), :] = val.astype(BF16)
                                jobs.append((store, head))
                _store_spread(jobs, tokens, _keep(t))

            lax.fori_loop(0, STEPS, queries_values, None)

        pl.run_scoped(
            project_a,
            pltpu.VMEM((S // 2, DM), U32), pltpu.VMEM((4, 4, DM // 8, DM), U32), pltpu.VMEM((S // 2, DC), U32),
            pltpu.VMEM((4, DM // 8, DM), U32), pltpu.VMEM((4, DM // 8, DM), U32),
            pltpu.VMEM((PRODUCTS, DM // 8, DM // 4), U32), pltpu.VMEM((2, 4, DM // 4, 8, D), U32),
            pltpu.SemaphoreType.DMA((5 * STEPS + 2,)))
        for copy in [bx_load] + kv_loads:
            copy.wait()

        def project_b(kv32):
            def window_attention(t, tokens):
                first = pl.multiple_of(t * ROWS, ROWS)
                for part in (1, 2):
                    for c in range(8):
                        kv32[part - 1, c] = qkv[part, c, pl.ds(first, A_HALO + ROWS), :].astype(F32)
                lane = lax.broadcasted_iota(jnp.int32, (8, 128), 1)
                sublane = lax.broadcasted_iota(jnp.int32, (8, 128), 0)
                keep = _keep(t)
                groups = ROWS // 8
                period = (len(tokens) / 2.5 - 32) / (groups + 1)

                def at(y, when):
                    return _after(y, tokens[min(int(when * 2.5), len(tokens) - 1)], keep)

                q = []
                for r in range(0, ROWS, 16):
                    both = [qkv[0, c, pl.ds(first + A_HALO + r, 16), :].astype(F32) for c in range(8)]
                    q += [[y[:8] for y in both], [y[8:] for y in both]]

                logits = [[None] * A_WINDOW for _ in range(groups)]
                for g in range(-1, groups):
                    r = A_HALO + 8 * g
                    k = [[kv32[0, c, r - n:r - n + 8, :] for n in (0, 2, 4, 6)] for c in range(8)]
                    for w in range(A_WINDOW):
                        if 0 <= g + w // 4 < groups:
                            logits[g + w // 4][w] = at(_sum([q[g + w // 4][c] * k[c][w % 4] for c in range(8)]),
                                                       (g + 1) * period + 2 * (w % 4) + w // 4)
                p = []
                for g in range(groups):
                    t0 = (g + 1) * period
                    x = logits[g]
                    for bit, lag in ((1, 6), (2, 12)):
                        x = [at(y + jnp.where((lane & bit) != 0, pltpu.roll(y, bit, 1), pltpu.roll(y, 128 - bit, 1)),
                                t0 + lag + (w + 4) % 8) for w, y in enumerate(x)]
                    x = [jnp.where(sublane + first + 8 * g >= 2 * w, y, MASKED) if 8 * g < 2 * w else y
                         for w, y in enumerate(x)]
                    top = x[0]
                    for y in x[1:]:
                        top = jnp.maximum(top, y)
                    x = [jnp.exp2(y - top) for y in x]
                    total = _sum(x)
                    inv = pl.reciprocal(total, approx=True)
                    inv = at(inv * (2.0 - total * inv), t0 + 21)
                    p.append([y * inv for y in x])
                out = [[None] * 8 for _ in range(groups)]
                for g in range(-1, groups):
                    r = A_HALO + 8 * g
                    for c in range(8):
                        before, now = kv32[1, c, r - 8:r, :], kv32[1, c, r:r + 8, :]
                        v = [now] + [pltpu.roll(jnp.where(sublane >= 8 - n, before, now), n, 0) for n in (2, 4, 6)]
                        when = (g + 2) * period + 12 + c
                        if g >= 0:
                            out[g][c] = at(out[g][c] + _sum([p[g][w] * v[w] for w in range(4)]), when)
                        if g + 1 < groups:
                            out[g + 1][c] = at(_sum([p[g + 1][4 + w] * v[w] for w in range(4)]), when)
                    if g > 0 and g % 2:
                        words = _head_shuffle([_pack(low, high) for low, high in zip(out[g - 1], out[g])],
                                              inverse=True)
                        rows = pl.ds(pl.multiple_of(first // 2 + 4 * (g - 1), 8), 8)
                        for c, y in enumerate(_chunks(words)):
                            mixed[rows, 128 * c:128 * (c + 1)] = at(y, (g + 2) * period + 24 + c)

            def queries(t, _):
                tokens = []
                lhs = _word_factors(bx[word_rows(t), :], _LHS)
                q = _strassen(lambda i: lhs[i],
                              lambda i: jnp.concatenate([wq_fac.bitcast(U32)[i, h] for h in range(H // 4)], axis=1),
                              _collect(tokens, 8, 256))
                for h, y in enumerate(_chunks(q * (D ** -0.5 * LOG2E))):
                    ctx[h, pl.ds(pl.multiple_of(t * ROWS, ROWS), ROWS), :] = y.astype(BF16)
                window_attention(t, tokens)
                _store_spread(list(kv_factors(0, [pl.multiple_of(t * 16, 16)])), tokens, _keep(t))

            lax.fori_loop(0, STEPS, queries, None)

        pl.run_scoped(project_b, pltpu.VMEM((2, 8, A_HALO + ROWS, 128), F32))

    pl.run_scoped(project, pltpu.VMEM((S // 2, DM), U32), pltpu.VMEM((3, 8, A_HALO + S, 128), BF16),
                  pltpu.VMEM((PRODUCTS, H // 4, DM // 4, D), BF16), pltpu.SemaphoreType.DMA)

    def attend(wob, wob_fac, result, sem):
        per_pair = H * D // 8 // (H // 2)

        def wob_copy(j):
            rows = pl.ds(pl.multiple_of(j * per_pair, per_pair), per_pair)
            return pltpu.make_async_copy(wob_hbm.bitcast(U32).at[:, rows, :], wob.at[j & 1], sem.at[j & 1])

        wob_copy(0).start()

        def head_pair(j, _):
            @pl.when(j + 1 < H // 2)
            def _():
                wob_copy(j + 1).start()

            wob_copy(j).wait()
            below = (lax.broadcasted_iota(jnp.int32, (TILE, TILE), 1)
                     <= lax.broadcasted_iota(jnp.int32, (TILE, TILE), 0))
            keep = _keep(j)
            ks, vs, scores, results, stored = {}, {}, {}, {}, []

            early = []
            for piece in range(0, per_pair, 8):
                start = pl.multiple_of(j * per_pair + piece, 8)
                words = jnp.concatenate([wob[j & 1, b, piece:piece + 8, :] for b in range(4)], axis=0)
                for i, y in enumerate(_word_factors(words, _RHS)):
                    def store(val, i=i, start=start):
                        wob_fac[i, pl.ds(start, 8), :] = val
                    early.append((store, y))
            late = list(kv_factors(jnp.minimum(j + 1, H // 2 - 1), range(0, DC // 4, 16)))

            tokens = []
            for chunk in range(S // CHUNK):
                kv = _strassen(lambda i: c_fac[chunk, i], lambda i: wkv_fac.bitcast(U32)[i],
                               _collect(tokens, 32, 128)).astype(BF16)
                for t in range(CHUNK // TILE):
                    k0, k1, v0, v1 = _chunks(kv[t * TILE:(t + 1) * TILE])
                    i = chunk * (CHUNK // TILE) + t
                    ks[0, i], ks[1, i], vs[0, i], vs[1, i] = k0, k1, v0, v1
            _store_spread(early, tokens, keep)
            tokens = []

            def score(e, i):
                q = ctx.bitcast(U32)[2 * j + e, i * TILE // 2:(i + 1) * TILE // 2, :]
                while stored:
                    e0, i0 = stored.pop()
                    token = ctx.bitcast(U32)[2 * j + e0 + (j >> 8), i0 * TILE // 2:i0 * TILE // 2 + 8, :]
                    q = jnp.concatenate([_after(q[:8], token, keep), q[8:]], axis=0)
                s = lax.dot_general(pltpu.bitcast(q, BF16),
                                    jnp.concatenate([ks[e, t] for t in range(i + 1)], axis=0),
                                    NT_DIMS, preferred_element_type=F32)
                _collect(tokens, 16, 512)(s)
                diagonal = jnp.where(below, s[:, i * TILE:], MASKED)
                s = jnp.concatenate([s[:, :i * TILE], diagonal], axis=1) if i else diagonal
                scores[e, i] = s, jnp.max(s, axis=1, keepdims=True)

            def context(e, i):
                s, top = scores.pop((e, i))
                p = jnp.exp2(s - top)
                total = jnp.sum(p, axis=1, keepdims=True)
                o = _dot(p.astype(BF16), jnp.concatenate([vs[e, t] for t in range(i + 1)], axis=0))
                inv = pl.reciprocal(total, approx=True)
                results[e, i] = (o * (inv * (2.0 - total * inv))).astype(BF16)

            def store_tile(e, i):
                ctx[2 * j + e, i * TILE:(i + 1) * TILE, :] = results.pop((e, i))
                stored.append((e, i))

            for name, tile in _attention_order(S // TILE):
                {"scores": score, "context": context, "store": store_tile}[name](*tile)
            _store_spread(late, tokens[len(tokens) // 10:len(tokens) * 8 // 10], keep)

        lax.fori_loop(0, H // 2, head_pair, None)

        def out_copy(t, side):
            rows = pl.ds(pl.multiple_of(t * ROWS, ROWS), ROWS)
            return pltpu.make_async_copy(result.at[side, t & 1], out_hbm.at[rows, pl.ds(side * DM, DM)],
                                         out_sem.at[2 * side + (t & 1)])

        def outputs(t, _):
            @pl.when(t >= 2)
            def _():
                out_copy(t - 2, 0).wait()
                out_copy(t - 2, 1).wait()

            lhs_b = _word_factors(jnp.concatenate([ctx.bitcast(U32)[h, word_rows(t), :] for h in range(H)], axis=1),
                                  _LHS)
            result[1, t & 1] = _strassen(lambda i: lhs_b[i], lambda i: wob_fac[i]).astype(BF16)
            low, high = _unpack(mixed[word_rows(t), :])
            o = jnp.concatenate([y[r:r + 8] for r in range(0, ROWS // 2, 8) for y in (low, high)], axis=0)
            lhs_a = [y.astype(BF16) for y in _f32_factors(o, _LHS)]
            products = []

            def send_b(prod):
                products.append(prod)
                if len(products) == 30:
                    out_copy(t, 1).start()

            result[0, t & 1] = _strassen(lambda i: lhs_a[i], lambda i: wo_fac[i], send_b).astype(BF16)
            out_copy(t, 0).start()

        lax.fori_loop(0, STEPS, outputs, None)
        for t in (STEPS - 2, STEPS - 1):
            out_copy(t, 0).wait()
            out_copy(t, 1).wait()

    pl.run_scoped(
        attend,
        pltpu.VMEM((2, 4, D // 4, DM), U32), pltpu.VMEM((PRODUCTS, H * D // 8, DM // 4), U32),
        pltpu.VMEM((2, 2, ROWS, DM), BF16), pltpu.SemaphoreType.DMA((2,)))


@jax.jit
def pallas_concat_heads__sliding_local_dilated__compressed_kv_cla__prompt_kernel(
    A_x: jax.Array,
    A_wqkv: jax.Array,
    A_wo: jax.Array,
    B_x: jax.Array,
    B_c_kv: jax.Array,
    B_w_q: jax.Array,
    B_w_uk: jax.Array,
    B_w_uv: jax.Array,
    B_w_o: jax.Array,
):
    assert A_x.shape == B_x.shape == (1, S, DM) and B_c_kv.shape == (1, S, DC)
    assert B_w_q.shape == (DM, H, D) and B_w_uk.shape == B_w_uv.shape == (DC, H, D)
    out = pl.pallas_call(
        _kernel,
        out_shape=jax.ShapeDtypeStruct((S, 2 * DM), BF16),
        in_specs=[pl.BlockSpec(memory_space=pl.ANY)] * 9,
        out_specs=pl.BlockSpec(memory_space=pl.ANY),
        scratch_shapes=[
            pltpu.VMEM((2, DC, 8, D), U32), pltpu.VMEM((2, DC, 8, D), U32),
            pltpu.VMEM((S // CHUNK, PRODUCTS, CHUNK // 8, DC // 4), U32),
            pltpu.VMEM((PRODUCTS, DC // 4, D), BF16), pltpu.VMEM((PRODUCTS, DM // 8, DM // 4), U32),
            pltpu.VMEM((H, S, D), BF16), pltpu.VMEM((S // 2, DM), U32),
            pltpu.SemaphoreType.DMA, pltpu.SemaphoreType.DMA((4,)),
        ],
        compiler_params=pltpu.CompilerParams(vmem_limit_bytes=126 * 1024 * 1024),
        name="concat_heads_attention",
    )(
        A_x.reshape(S, DM), A_wqkv.reshape(4, DM // 4, 3 * DM), A_wo.reshape(4, DM // 4, DM),
        B_x.reshape(S, DM), B_c_kv.reshape(S, DC), B_w_q.reshape(4, DM // 4, H, D), B_w_uk, B_w_uv,
        B_w_o.reshape(4, H * D // 4, DM),
    )
    return out.reshape(1, S, 2 * DM)
```

```python
import math

import jax
import jax.numpy as jnp
from jax import lax
import jax.experimental.pallas as pl
import jax.experimental.pallas.tpu as pltpu

F32, BF16, U32 = jnp.float32, jnp.bfloat16, jnp.uint32
LOG2E = math.log2(math.e)
NT_DIMS = (((1,), (1,)), ((), ()))
MASKED = -1e30

S, DM = 2048, 1024
A_DH, A_WINDOW = 32, 8
A_HALO = 16
H, D, DC = 32, 128, 512
ROWS = 256
STEPS = S // ROWS
CHUNK = 1024
TILE = 128
LEVELS = 2
PRODUCTS = 7 ** LEVELS
O_LEVELS = 3


def _unpack(words):
    return pltpu.bitcast(words << 16, F32), pltpu.bitcast(words & jnp.uint32(0xFFFF0000), F32)


def _pack(low, high):
    return pltpu.pack_elementwise([low, high], packed_dtype=BF16)


def _chunks(x):
    return [x[:, c:c + 128] for c in range(0, x.shape[1], 128)]


_LHS = ((0, 3, 1), (2, 3, 1), (0, None, 0), (3, None, 0), (0, 1, 1), (2, 0, -1), (1, 3, -1))
_RHS = ((0, 3, 1), (0, None, 0), (1, 3, -1), (2, 0, -1), (3, None, 0), (0, 1, 1), (2, 3, 1))


def _quadrants(x):
    m, n = x.shape[0] // 2, x.shape[1] // 2
    return x[:m, :n], x[:m, n:], x[m:, :n], x[m:, n:]


def _factors(parts, words, levels, recipe, first=None):
    if levels == 0:
        return [(parts, words)]
    quads = list(zip(*[_quadrants(p) for p in parts]))
    out = []
    for a, b, sign in recipe if first is None else [recipe[first]]:
        if b is None:
            out += _factors(quads[a], None if words is None else _quadrants(words)[a], levels - 1, recipe)
        else:
            mixed = [x + y if sign > 0 else x - y for x, y in zip(quads[a], quads[b])]
            out += _factors(mixed, None, levels - 1, recipe)
    return out


def _word_factors(words, recipe, levels=LEVELS, first=None):
    return [_pack(*parts) if plain is None else plain
            for parts, plain in _factors(_unpack(words), words, levels, recipe, first)]


def _f32_factors(x, recipe):
    return [y for (y,), _ in _factors([x], None, LEVELS, recipe)]


def _dot(a, b):
    a, b = [y if y.dtype == BF16 else pltpu.bitcast(y, BF16) for y in (a, b)]
    return jnp.dot(a, b, preferred_element_type=F32)


def _strassen(lhs, rhs, watch=None, levels=LEVELS, base=0):
    if levels == 0:
        out = _dot(lhs(base), rhs(base))
        if watch is not None:
            watch(out)
        return out
    step = 7 ** (levels - 1)
    m3, m4, m5, m2, m1, m6, m7 = [_strassen(lhs, rhs, watch, levels - 1, base + i * step)
                                  for i in (2, 3, 4, 1, 0, 5, 6)]
    return jnp.concatenate([jnp.concatenate([m4 - m5 + m1 + m7, m3 + m5], axis=1),
                            jnp.concatenate([m2 + m4, m3 - m2 + m1 + m6], axis=1)], axis=0)


def _slab(load, total, start, n):
    return jnp.concatenate([load(total // 4 * b + start, n) for b in range(4)], axis=0)


def _keep(step):
    return lax.broadcasted_iota(jnp.int32, (8, 128), 1) + step >= 0


def _after(x, token, keep):
    return jnp.where(keep, x, pltpu.bitcast(token, x.dtype))


def _collect(tokens, row_step, col_step):
    return lambda prod: tokens.extend(prod[r:r + 8, c:c + 128] for c in range(0, prod.shape[1], col_step)
                                      for r in range(0, prod.shape[0], row_step))


def _store_spread(jobs, tokens, keep):
    def height(val):
        return 8 if val.dtype == U32 else 16

    total = sum(val.size // (128 * height(val)) for _, val in jobs)
    n = 0
    for store, val in jobs:
        rows = []
        for r in range(0, val.shape[0], height(val)):
            cols = []
            for piece in _chunks(val[r:r + 8]):
                cols.append(_after(piece, tokens[n * len(tokens) // total], keep))
                n += 1
            rows.append(jnp.concatenate(cols, axis=1))
            if height(val) == 16:
                rows.append(val[r + 8:r + 16])
        store(jnp.concatenate(rows, axis=0))


def _head_shuffle(chunks, inverse=False):
    group = (lax.broadcasted_iota(jnp.int32, chunks[0].shape, 1) >> 2) & 7

    def rotate(x, c):
        if c == 0:
            return x
        if inverse:
            return jnp.where(group >= c, pltpu.roll(x, 4 * c, 1), pltpu.roll(x, 96 + 4 * c, 1))
        return jnp.where(group < 8 - c, pltpu.roll(x, 128 - 4 * c, 1), pltpu.roll(x, 32 - 4 * c, 1))

    def exchange(xs):
        xs = [xs[-c % 8] for c in range(8)]
        for bit in (1, 2, 4):
            xs = [jnp.where((group & bit) != 0, xs[(c - bit) % 8], xs[c]) for c in range(8)]
        return xs

    if inverse:
        return jnp.concatenate(exchange([rotate(x, c) for c, x in enumerate(chunks)]), axis=1)
    return jnp.concatenate([rotate(x, c) for c, x in enumerate(exchange(chunks))], axis=1)


def _attention_order(n_tiles, lead=8, hold=3):
    tiles = [(e, i) for i in reversed(range(n_tiles)) for e in range(2)]
    steps, done = [], 0
    for t, tile in enumerate(tiles):
        steps.append(("scores", tile))
        while sum(i + 1 for _, i in tiles[done + 1:t + 1]) >= lead:
            steps.append(("context", tiles[done]))
            if done >= hold:
                steps.append(("store", tiles[done - hold]))
            done += 1
    steps += [("context", tile) for tile in tiles[done:]]
    steps += [("store", tile) for tile in tiles[done - hold:]]
    return steps


def _sum(terms):
    return sum(terms[1:], terms[0])


def _kernel(ax_hbm, wqkv_hbm, wo_hbm, bx_hbm, c_hbm, wq_hbm, wuk_hbm, wuv_hbm, wob_hbm, out_hbm,
            wkv_raw, c_fac, wkv_fac, wo_fac, ctx, mixed, in_sem, out_sem):
    def kv_copies(j):
        return [pltpu.make_async_copy(src.bitcast(U32).at[:, j, 0, :], wkv_raw.at[j & 1, i], in_sem.at[j & 1])
                for i, src in enumerate((wuk_hbm, wuv_hbm))]

    def kv_factors(j, starts):
        def load(start, n):
            return jnp.concatenate([y for i in range(2) for y in _unpack(wkv_raw[j & 1, i, pl.ds(start, n), :])],
                                   axis=1)

        for start in starts:
            for i, y in enumerate(_f32_factors(_slab(load, DC, start, 16), _RHS)):
                def store(val, i=i, start=start):
                    wkv_fac[i, pl.ds(start, 16), :] = val.astype(BF16)
                yield store, y

    def word_rows(t):
        return pl.ds(pl.multiple_of(t * (ROWS // 2), ROWS // 2), ROWS // 2)

    def project(bx, qkv, wq_fac, bx_sem):
        bx_load = pltpu.make_async_copy(bx_hbm.bitcast(U32), bx, bx_sem)

        def project_a(ax, w_raw, cc, q_w, k_w, v_fac, wq_raw, sem):
            slab = DM // 8 // STEPS

            def weight_copy(part, t):
                rows = pl.ds(t * slab, slab)
                return pltpu.make_async_copy(wqkv_hbm.bitcast(U32).at[:, rows, pl.ds(part * DM, DM)],
                                             w_raw.at[part, :, rows, :], sem.at[part * STEPS + t])

            def x_copy(t):
                rows = pl.ds(t * (ROWS // 2), ROWS // 2)
                return pltpu.make_async_copy(ax_hbm.bitcast(U32).at[rows], ax.at[rows], sem.at[3 * STEPS + t])

            def wq_copies(t):
                rows = pl.ds((t & 1) * (DM // 8), DM // 8)
                return [pltpu.make_async_copy(wq_hbm.bitcast(U32).at[:, rows, 4 * b + (t >> 1), 0, :],
                                              wq_raw.at[t, b], sem.at[4 * STEPS + t]) for b in range(4)]

            later_loads = [pltpu.make_async_copy(src.bitcast(U32), dst, sem.at[5 * STEPS + i])
                           for i, (src, dst) in enumerate(((wo_hbm, w_raw.at[3]), (c_hbm, cc)))]
            for t in range(STEPS):
                weight_copy(1, t).start()
            for t in range(STEPS):
                for copy in (x_copy(t), weight_copy(0, t), weight_copy(2, t)):
                    copy.start()
            for copy in later_loads:
                copy.start()

            def weights(part, t):
                rows = pl.ds(pl.multiple_of(t * slab, slab), slab)
                quarters = [w_raw[part, b, rows, :] for b in range(4)]
                if part < 3:
                    quarters = [_head_shuffle(_chunks(w)) for w in quarters]
                if part >= 2:
                    quarters = _word_factors(jnp.concatenate(quarters, axis=0), _RHS)
                for i, y in enumerate(quarters):
                    def store(val, i=i):
                        (q_w, k_w, v_fac, wo_fac)[part][i, rows, :] = val
                    yield store, y

            def prepare_keys(t, _):
                weight_copy(1, t).wait()
                for store, words in weights(1, t):
                    store(words)

            lax.fori_loop(0, STEPS, prepare_keys, None)
            for t in range(STEPS):
                for copy in wq_copies(t):
                    copy.start()
            for copy in [bx_load] + kv_copies(0) + kv_copies(1):
                copy.start()
            qkv[1:, :, :A_HALO, :] = jnp.zeros((2, 8, A_HALO, 128), BF16)

            def project_rows(part, t, tokens):
                x = ax[word_rows(t), :]
                if part < 2:
                    out = _dot(x, jnp.concatenate([(q_w, k_w)[part][b] for b in range(4)], axis=0))
                    _collect(tokens, 8, 128)(out)
                else:
                    lhs = _word_factors(x, _LHS)
                    out = _strassen(lambda i: lhs[i], lambda i: v_fac[i], _collect(tokens, 32, 256))
                if part == 0:
                    out = out * (A_DH ** -0.5 * LOG2E)
                for c, y in enumerate(_chunks(out)):
                    qkv[part, c, pl.ds(pl.multiple_of(t * ROWS + A_HALO, A_HALO), ROWS), :] = y.astype(BF16)

            def keys(t, _):
                for copy in (x_copy(t), weight_copy(0, t), weight_copy(2, t)):
                    copy.wait()
                tokens = []
                project_rows(1, t, tokens)
                _store_spread([*weights(0, t), *weights(2, t)], tokens, _keep(t))

            lax.fori_loop(0, STEPS, keys, None)
            for copy in later_loads:
                copy.wait()

            def queries_values(t, _):
                for copy in wq_copies(t):
                    copy.wait()
                tokens = []
                project_rows(0, t, tokens)
                project_rows(2, t, tokens)
                jobs = list(weights(3, t))
                per_chunk = STEPS // (S // CHUNK)
                n = CHUNK // 8 // per_chunk
                chunk, start = t // per_chunk, pl.multiple_of((t % per_chunk) * n, n)
                words = _slab(lambda row, m: cc[pl.ds(pl.multiple_of(chunk * (CHUNK // 2) + row, m), m), :],
                              CHUNK // 2, start, n)
                for i, y in enumerate(_word_factors(words, _LHS)):
                    def store(val, i=i):
                        c_fac[chunk, i, pl.ds(start, n), :] = val
                    jobs.append((store, y))
                for piece in range(0, DM // 8, 16):
                    first = pl.multiple_of((t & 1) * (DM // 8) + piece, 16)
                    w = jnp.concatenate([jnp.concatenate(
                        [y for b in range(4) for y in _unpack(wq_raw[t, b, quarter, piece:piece + 16, :])], axis=1)
                        for quarter in range(4)], axis=0)
                    for i, y in enumerate(_f32_factors(w, _RHS)):
                        for e, head in enumerate(_chunks(y)):
                            def store(val, i=i, slot=(t >> 1) * 2 + e, first=first):
                                wq_fac[i, slot, pl.ds(first, 16), :] = val.astype(BF16)
                            jobs.append((store, head))
                _store_spread(jobs, tokens, _keep(t))

            lax.fori_loop(0, STEPS, queries_values, None)

        pl.run_scoped(
            project_a,
            pltpu.VMEM((S // 2, DM), U32), pltpu.VMEM((4, 4, DM // 8, DM), U32), pltpu.VMEM((S // 2, DC), U32),
            pltpu.VMEM((4, DM // 8, DM), U32), pltpu.VMEM((4, DM // 8, DM), U32),
            pltpu.VMEM((PRODUCTS, DM // 8, DM // 4), U32), pltpu.VMEM((STEPS, 4, 4, DM // 8, D), U32),
            pltpu.SemaphoreType.DMA((5 * STEPS + 2,)))
        for copy in [bx_load] + kv_copies(0):
            copy.wait()

        def project_b(kv32):
            def window_attention(t, tokens):
                first = pl.multiple_of(t * ROWS, ROWS)
                for part in (1, 2):
                    for c in range(8):
                        kv32[part - 1, c] = qkv[part, c, pl.ds(first, A_HALO + ROWS), :].astype(F32)
                lane = lax.broadcasted_iota(jnp.int32, (8, 128), 1)
                sublane = lax.broadcasted_iota(jnp.int32, (8, 128), 0)
                keep = _keep(t)
                groups = ROWS // 8
                period = (len(tokens) / 2.5 - 32) / (groups + 1)

                def at(y, when):
                    return _after(y, tokens[min(int(when * 2.5), len(tokens) - 1)], keep)

                q = []
                for r in range(0, ROWS, 16):
                    both = [qkv[0, c, pl.ds(first + A_HALO + r, 16), :].astype(F32) for c in range(8)]
                    q += [[y[:8] for y in both], [y[8:] for y in both]]

                logits = [[None] * A_WINDOW for _ in range(groups)]
                for g in range(-1, groups):
                    r = A_HALO + 8 * g
                    k = [[kv32[0, c, r - n:r - n + 8, :] for n in (0, 2, 4, 6)] for c in range(8)]
                    for w in range(A_WINDOW):
                        if 0 <= g + w // 4 < groups:
                            logits[g + w // 4][w] = at(_sum([q[g + w // 4][c] * k[c][w % 4] for c in range(8)]),
                                                       (g + 1) * period + 2 * (w % 4) + w // 4)
                p = []
                for g in range(groups):
                    t0 = (g + 1) * period
                    x = logits[g]
                    for bit, lag in ((1, 6), (2, 12)):
                        x = [at(y + jnp.where((lane & bit) != 0, pltpu.roll(y, bit, 1), pltpu.roll(y, 128 - bit, 1)),
                                t0 + lag + (w + 4) % 8) for w, y in enumerate(x)]
                    x = [jnp.where(sublane + first + 8 * g >= 2 * w, y, MASKED) if 8 * g < 2 * w else y
                         for w, y in enumerate(x)]
                    top = x[0]
                    for y in x[1:]:
                        top = jnp.maximum(top, y)
                    x = [jnp.exp2(y - top) for y in x]
                    total = _sum(x)
                    inv = pl.reciprocal(total, approx=True)
                    inv = at(inv * (2.0 - total * inv), t0 + 21)
                    p.append([y * inv for y in x])
                out = [[None] * 8 for _ in range(groups)]
                for g in range(-1, groups):
                    r = A_HALO + 8 * g
                    for c in range(8):
                        before, now = kv32[1, c, r - 8:r, :], kv32[1, c, r:r + 8, :]
                        v = [now] + [pltpu.roll(jnp.where(sublane >= 8 - n, before, now), n, 0) for n in (2, 4, 6)]
                        when = (g + 2) * period + 12 + c
                        if g >= 0:
                            out[g][c] = at(out[g][c] + _sum([p[g][w] * v[w] for w in range(4)]), when)
                        if g + 1 < groups:
                            out[g + 1][c] = at(_sum([p[g + 1][4 + w] * v[w] for w in range(4)]), when)
                    if g > 0 and g % 2:
                        words = _head_shuffle([_pack(low, high) for low, high in zip(out[g - 1], out[g])],
                                              inverse=True)
                        rows = pl.ds(pl.multiple_of(first // 2 + 4 * (g - 1), 8), 8)
                        for c, y in enumerate(_chunks(words)):
                            mixed[rows, 128 * c:128 * (c + 1)] = at(y, (g + 2) * period + 24 + c)

            def queries(t, _):
                tokens = []
                lhs = _word_factors(bx[word_rows(t), :], _LHS)
                q = _strassen(lambda i: lhs[i],
                              lambda i: jnp.concatenate([wq_fac.bitcast(U32)[i, h] for h in range(H // 4)], axis=1),
                              _collect(tokens, 8, 256))
                for h, y in enumerate(_chunks(q * (D ** -0.5 * LOG2E))):
                    ctx[h, pl.ds(pl.multiple_of(t * ROWS, ROWS), ROWS), :] = y.astype(BF16)
                window_attention(t, tokens)
                _store_spread(list(kv_factors(0, [pl.multiple_of(t * 16, 16)])), tokens, _keep(t))

            lax.fori_loop(0, STEPS, queries, None)

        pl.run_scoped(project_b, pltpu.VMEM((2, 8, A_HALO + ROWS, 128), F32))

    pl.run_scoped(project, pltpu.VMEM((S // 2, DM), U32), pltpu.VMEM((3, 8, A_HALO + S, 128), BF16),
                  pltpu.VMEM((PRODUCTS, H // 4, DM // 4, D), BF16), pltpu.SemaphoreType.DMA)

    def attend(wob, wob_fac, result, sem):
        per_pair = D >> O_LEVELS

        def wob_copy(j):
            rows = pl.ds(pl.multiple_of(j * per_pair, per_pair), per_pair)
            return pltpu.make_async_copy(wob_hbm.bitcast(U32).at[:, rows, :], wob.at[j & 1], sem.at[j & 1])

        wob_copy(0).start()

        def head_pair(j, _):
            @pl.when(j + 1 < H // 2)
            def _():
                wob_copy(j + 1).start()
                for copy in kv_copies(j + 1):
                    copy.wait()

            @pl.when(j + 2 < H // 2)
            def _():
                for copy in kv_copies(j + 2):
                    copy.start()

            wob_copy(j).wait()
            below = (lax.broadcasted_iota(jnp.int32, (TILE, TILE), 1)
                     <= lax.broadcasted_iota(jnp.int32, (TILE, TILE), 0))
            keep = _keep(j)
            ks, vs, scores, results, stored = {}, {}, {}, {}, []

            early = []
            for piece in range(0, per_pair, 8):
                start = pl.multiple_of(j * per_pair + piece, 8)
                words = jnp.concatenate([wob[j & 1, b, piece:piece + 8, :] for b in range(2 ** O_LEVELS)], axis=0)
                for i, y in enumerate(_word_factors(words, _RHS, O_LEVELS)):
                    def store(val, i=i, start=start):
                        wob_fac[i, pl.ds(start, 8), :] = val
                    early.append((store, y))
            late = list(kv_factors(j + 1, range(0, DC // 4, 16)))

            tokens = []
            for chunk in range(S // CHUNK):
                kv = _strassen(lambda i: c_fac[chunk, i], lambda i: wkv_fac.bitcast(U32)[i],
                               _collect(tokens, 32, 128)).astype(BF16)
                for t in range(CHUNK // TILE):
                    k0, k1, v0, v1 = _chunks(kv[t * TILE:(t + 1) * TILE])
                    i = chunk * (CHUNK // TILE) + t
                    ks[0, i], ks[1, i], vs[0, i], vs[1, i] = k0, k1, v0, v1
            _store_spread(early[:len(early) * 7 // 10], tokens[:len(tokens) * 9 // 10], keep)
            late += early[len(early) * 7 // 10:]
            tokens = []

            def score(e, i):
                q = ctx.bitcast(U32)[2 * j + e, i * TILE // 2:(i + 1) * TILE // 2, :]
                while stored:
                    e0, i0 = stored.pop()
                    token = ctx.bitcast(U32)[2 * j + e0 + (j >> 8), i0 * TILE // 2:i0 * TILE // 2 + 8, :]
                    q = jnp.concatenate([_after(q[:8], token, keep), q[8:]], axis=0)
                s = lax.dot_general(pltpu.bitcast(q, BF16),
                                    jnp.concatenate([ks[e, t] for t in range(i + 1)], axis=0),
                                    NT_DIMS, preferred_element_type=F32)
                _collect(tokens, 16, 512)(s)
                diagonal = jnp.where(below, s[:, i * TILE:], MASKED)
                s = jnp.concatenate([s[:, :i * TILE], diagonal], axis=1) if i else diagonal
                scores[e, i] = s, jnp.max(s, axis=1, keepdims=True)

            def context(e, i):
                s, top = scores.pop((e, i))
                p, total = _chunks(jnp.exp2(s - top)), None
                for t in range(0, i + 1, 2):
                    last = min(t + 1, i)
                    total = _sum(p[t:t + 2]) if total is None else total + _sum(p[t:t + 2])
                    p[last] = jnp.concatenate(
                        [_after(p[last][r:r + 8], total[r:r + 8], keep) if r % 32 == 24 else p[last][r:r + 8]
                         for r in range(0, TILE, 8)], axis=0)
                total = jnp.sum(total, axis=1, keepdims=True)
                o = _dot(jnp.concatenate(p, axis=1).astype(BF16),
                         jnp.concatenate([vs[e, t] for t in range(i + 1)], axis=0))
                inv = pl.reciprocal(total, approx=True)
                results[e, i] = (o * (inv * (2.0 - total * inv))).astype(BF16)

            def store_tile(e, i):
                ctx[2 * j + e, i * TILE:(i + 1) * TILE, :] = results.pop((e, i))
                stored.append((e, i))

            for name, tile in _attention_order(S // TILE):
                {"scores": score, "context": context, "store": store_tile}[name](*tile)
            _store_spread(late, tokens[len(tokens) // 10:len(tokens) * 8 // 10], keep)

        lax.fori_loop(0, H // 2, head_pair, None)

        def out_copy(t, side):
            rows = pl.ds(pl.multiple_of(t * ROWS, ROWS), ROWS)
            return pltpu.make_async_copy(result.at[side, t & 1], out_hbm.at[rows, pl.ds(side * DM, DM)],
                                         out_sem.at[2 * side + (t & 1)])

        def outputs(t, _):
            @pl.when(t >= 2)
            def _():
                out_copy(t - 2, 0).wait()
                out_copy(t - 2, 1).wait()

            lhs_b = []
            for g in range(7):
                rows = word_rows(t + (t >> (8 + g)))
                words = jnp.concatenate([ctx.bitcast(U32)[h, rows, :] for h in range(H)], axis=1)
                lhs_b += _word_factors(words, _LHS, O_LEVELS, g)
            result[1, t & 1] = _strassen(lambda i: lhs_b[i], lambda i: wob_fac[i], None, O_LEVELS).astype(BF16)
            low, high = _unpack(mixed[word_rows(t), :])
            o = jnp.concatenate([y[r:r + 8] for r in range(0, ROWS // 2, 8) for y in (low, high)], axis=0)
            lhs_a = [y.astype(BF16) for y in _f32_factors(o, _LHS)]
            products = []

            def send_b(prod):
                products.append(prod)
                if len(products) == 30:
                    out_copy(t, 1).start()

            result[0, t & 1] = _strassen(lambda i: lhs_a[i], lambda i: wo_fac[i], send_b).astype(BF16)
            out_copy(t, 0).start()

        lax.fori_loop(0, STEPS, outputs, None)
        for t in (STEPS - 2, STEPS - 1):
            out_copy(t, 0).wait()
            out_copy(t, 1).wait()

    pl.run_scoped(
        attend,
        pltpu.VMEM((2, 2 ** O_LEVELS, D >> O_LEVELS, DM), U32),
        pltpu.VMEM((7 ** O_LEVELS, H * D // 2 >> O_LEVELS, DM >> O_LEVELS), U32),
        pltpu.VMEM((2, 2, ROWS, DM), BF16), pltpu.SemaphoreType.DMA((2,)))


@jax.jit
def pallas_concat_heads__sliding_local_dilated__compressed_kv_cla__prompt_kernel(
    A_x: jax.Array,
    A_wqkv: jax.Array,
    A_wo: jax.Array,
    B_x: jax.Array,
    B_c_kv: jax.Array,
    B_w_q: jax.Array,
    B_w_uk: jax.Array,
    B_w_uv: jax.Array,
    B_w_o: jax.Array,
):
    assert A_x.shape == B_x.shape == (1, S, DM) and B_c_kv.shape == (1, S, DC)
    assert B_w_q.shape == (DM, H, D) and B_w_uk.shape == B_w_uv.shape == (DC, H, D)
    out = pl.pallas_call(
        _kernel,
        out_shape=jax.ShapeDtypeStruct((S, 2 * DM), BF16),
        in_specs=[pl.BlockSpec(memory_space=pl.ANY)] * 9,
        out_specs=pl.BlockSpec(memory_space=pl.ANY),
        scratch_shapes=[
            pltpu.VMEM((2, 2, DC, D), U32),
            pltpu.VMEM((S // CHUNK, PRODUCTS, CHUNK // 8, DC // 4), U32),
            pltpu.VMEM((PRODUCTS, DC // 4, D), BF16), pltpu.VMEM((PRODUCTS, DM // 8, DM // 4), U32),
            pltpu.VMEM((H, S, D), BF16), pltpu.VMEM((S // 2, DM), U32),
            pltpu.SemaphoreType.DMA((2,)), pltpu.SemaphoreType.DMA((4,)),
        ],
        compiler_params=pltpu.CompilerParams(vmem_limit_bytes=120 * 1024 * 1024),
        name="concat_heads_attention",
    )(
        A_x.reshape(S, DM), A_wqkv.reshape(4, DM // 4, 3 * DM), A_wo.reshape(4, DM // 4, DM),
        B_x.reshape(S, DM), B_c_kv.reshape(S, DC), B_w_q.reshape(4, DM // 4, H // 2, 2, D),
        B_w_uk.reshape(DC, H // 2, 2, D), B_w_uv.reshape(DC, H // 2, 2, D),
        B_w_o.reshape(2 ** O_LEVELS, H * D >> O_LEVELS, DM),
    )
    return out.reshape(1, S, 2 * DM)
```

```python
import math

import jax
import jax.numpy as jnp
from jax import lax
import jax.experimental.pallas as pl
import jax.experimental.pallas.tpu as pltpu

F32, BF16, U32 = jnp.float32, jnp.bfloat16, jnp.uint32
LOG2E = math.log2(math.e)
NT_DIMS = (((1,), (1,)), ((), ()))
MASKED = -1e30

S, DM = 2048, 1024
A_DH, A_WINDOW = 32, 8
A_HALO = 16
H, D, DC = 32, 128, 512
ROWS = 256
STEPS = S // ROWS
CHUNK = 1024
TILE = 128
LEVELS = 2
PRODUCTS = 7 ** LEVELS
O_LEVELS = 3


def _unpack(words):
    return pltpu.bitcast(words << 16, F32), pltpu.bitcast(words & jnp.uint32(0xFFFF0000), F32)


def _chunks(x):
    return [x[:, c:c + 128] for c in range(0, x.shape[1], 128)]


_LHS = ((0, 3, 1), (2, 3, 1), (0, None, 0), (3, None, 0), (0, 1, 1), (2, 0, -1), (1, 3, -1))
_RHS = ((0, 3, 1), (0, None, 0), (1, 3, -1), (2, 0, -1), (3, None, 0), (0, 1, 1), (2, 3, 1))


def _quadrants(x):
    m, n = x.shape[0] // 2, x.shape[1] // 2
    return x[:m, :n], x[:m, n:], x[m:, :n], x[m:, n:]


def _factors(x, recipe, levels=LEVELS, first=None):
    def split(wide, plain, levels, rows):
        if levels == 0:
            return [wide if plain is None else plain]
        quads, out = _quadrants(wide), []
        for a, b, sign in rows:
            if b is None:
                out += split(quads[a], None if plain is None else _quadrants(plain)[a], levels - 1, recipe)
            else:
                out += split(quads[a] + quads[b] if sign > 0 else quads[a] - quads[b], None, levels - 1, recipe)
        return out

    if x.dtype == U32:
        x = pltpu.bitcast(x, BF16)
    return split(x.astype(F32), x, levels, recipe if first is None else [recipe[first]])


def _dot(a, b):
    a, b = [pltpu.bitcast(y, BF16) if y.dtype == U32 else y.astype(BF16) for y in (a, b)]
    return jnp.dot(a, b, preferred_element_type=F32)


def _strassen(lhs, rhs, watch=None, levels=LEVELS, base=0):
    if levels == 0:
        out = _dot(lhs(base), rhs(base))
        if watch is not None:
            watch(out)
        return out
    step = 7 ** (levels - 1)
    m3, m4, m5, m2, m1, m6, m7 = [_strassen(lhs, rhs, watch, levels - 1, base + i * step)
                                  for i in (2, 3, 4, 1, 0, 5, 6)]
    return jnp.concatenate([jnp.concatenate([m4 - m5 + m1 + m7, m3 + m5], axis=1),
                            jnp.concatenate([m2 + m4, m3 - m2 + m1 + m6], axis=1)], axis=0)


def _wide(fac, i):
    return jnp.concatenate([fac.bitcast(U32)[i, c] for c in range(fac.shape[1])], axis=1)


def _slab(load, total, start, n):
    return jnp.concatenate([load(total // 4 * b + start, n) for b in range(4)], axis=0)


def _keep(step):
    return lax.broadcasted_iota(jnp.int32, (8, 128), 1) + step >= 0


def _after(x, token, keep):
    return jnp.where(keep, x, pltpu.bitcast(token, x.dtype))


def _collect(tokens, row_step, col_step):
    return lambda prod: tokens.extend(prod[r:r + 8, c:c + 128] for c in range(0, prod.shape[1], col_step)
                                      for r in range(0, prod.shape[0], row_step))


def _store_spread(jobs, tokens, keep):
    def height(val):
        return 8 if val.dtype == U32 else 16

    jobs = [(store, val.astype(F32) if val.dtype == BF16 else val) for store, val in jobs]
    total = sum(val.size // (128 * height(val)) for _, val in jobs)
    n = 0
    for store, val in jobs:
        rows = []
        for r in range(0, val.shape[0], height(val)):
            cols = []
            for piece in _chunks(val[r:r + 8]):
                cols.append(_after(piece, tokens[n * len(tokens) // total], keep))
                n += 1
            rows.append(jnp.concatenate(cols, axis=1))
            if height(val) == 16:
                rows.append(val[r + 8:r + 16])
        store(jnp.concatenate(rows, axis=0))


def _head_shuffle(chunks, inverse=False):
    group = (lax.broadcasted_iota(jnp.int32, chunks[0].shape, 1) >> 2) & 7

    def rotate(x, c):
        if c == 0:
            return x
        if inverse:
            return jnp.where(group >= c, pltpu.roll(x, 4 * c, 1), pltpu.roll(x, 96 + 4 * c, 1))
        return jnp.where(group < 8 - c, pltpu.roll(x, 128 - 4 * c, 1), pltpu.roll(x, 32 - 4 * c, 1))

    def exchange(xs):
        xs = [xs[-c % 8] for c in range(8)]
        for bit in (1, 2, 4):
            xs = [jnp.where((group & bit) != 0, xs[(c - bit) % 8], xs[c]) for c in range(8)]
        return xs

    if inverse:
        return jnp.concatenate(exchange([rotate(x, c) for c, x in enumerate(chunks)]), axis=1)
    return jnp.concatenate([rotate(x, c) for c, x in enumerate(exchange(chunks))], axis=1)


def _attention_order(n_tiles, lead=8, hold=3):
    tiles = [(e, i) for i in reversed(range(n_tiles)) for e in range(2)]
    steps, done = [], 0
    for t, tile in enumerate(tiles):
        steps.append(("scores", tile))
        while sum(i + 1 for _, i in tiles[done + 1:t + 1]) >= lead:
            steps.append(("context", tiles[done]))
            if done >= hold:
                steps.append(("store", tiles[done - hold]))
            done += 1
    steps += [("context", tile) for tile in tiles[done:]]
    steps += [("store", tile) for tile in tiles[done - hold:]]
    return steps


def _sum(terms):
    return sum(terms[1:], terms[0])


def _kernel(ax_hbm, wqkv_hbm, wo_hbm, bx_hbm, c_hbm, wq_hbm, wuk_hbm, wuv_hbm, wob_hbm, out_hbm,
            wkv_raw, c_fac, wkv_fac, wo_fac, ctx, mixed, in_sem, out_sem):
    def kv_copies(j):
        return [pltpu.make_async_copy(src.bitcast(U32).at[:, j, 0, :], wkv_raw.at[j & 1, i], in_sem.at[j & 1])
                for i, src in enumerate((wuk_hbm, wuv_hbm))]

    def kv_factors(j, starts):
        def load(start, n):
            return jnp.concatenate([y for i in range(2) for y in _unpack(wkv_raw[j & 1, i, pl.ds(start, n), :])],
                                   axis=1)

        for start in starts:
            for i, y in enumerate(_factors(_slab(load, DC, start, 16), _RHS)):
                def store(val, i=i, start=start):
                    wkv_fac[i, pl.ds(start, 16), :] = val.astype(BF16)
                yield store, y

    def word_rows(t):
        return pl.ds(pl.multiple_of(t * (ROWS // 2), ROWS // 2), ROWS // 2)

    def project(bx, qkv, wq_fac, bx_sem):
        bx_load = pltpu.make_async_copy(bx_hbm.bitcast(U32), bx, bx_sem)

        def project_a(ax, w_raw, cc, q_w, k_w, v_fac, wq_raw, sem):
            slab = DM // 8 // STEPS

            def weight_copy(part, t):
                rows = pl.ds(t * slab, slab)
                return pltpu.make_async_copy(wqkv_hbm.bitcast(U32).at[:, rows, pl.ds(part * DM, DM)],
                                             w_raw.at[part, :, rows, :], sem.at[part * STEPS + t])

            def x_copy(t):
                rows = pl.ds(t * (ROWS // 2), ROWS // 2)
                return pltpu.make_async_copy(ax_hbm.bitcast(U32).at[rows], ax.at[rows], sem.at[3 * STEPS + t])

            def wq_copies(t):
                rows = pl.ds((t & 1) * (DM // 8), DM // 8)
                return [pltpu.make_async_copy(wq_hbm.bitcast(U32).at[:, rows, 4 * b + (t >> 1), 0, :],
                                              wq_raw.at[t, b], sem.at[4 * STEPS + t]) for b in range(4)]

            later_loads = [pltpu.make_async_copy(src.bitcast(U32), dst, sem.at[5 * STEPS + i])
                           for i, (src, dst) in enumerate(((wo_hbm, w_raw.at[3]), (c_hbm, cc)))]
            for t in range(STEPS):
                weight_copy(1, t).start()
            for t in range(STEPS):
                for copy in (x_copy(t), weight_copy(0, t), weight_copy(2, t)):
                    copy.start()
            for copy in later_loads:
                copy.start()

            def weights(part, t):
                rows = pl.ds(pl.multiple_of(t * slab, slab), slab)
                quarters = [w_raw[part, b, rows, :] for b in range(4)]
                if part < 3:
                    quarters = [_head_shuffle(_chunks(w)) for w in quarters]
                if part >= 2:
                    quarters = _factors(jnp.concatenate(quarters, axis=0), _RHS)
                for i, y in enumerate(quarters):
                    def store(val, i=i):
                        if part < 2:
                            (q_w, k_w)[part][i, rows, :] = val
                        else:
                            for c, piece in enumerate(_chunks(val)):
                                target = pl.ds(pl.multiple_of(t * 2 * slab, 2 * slab), 2 * slab)
                                (v_fac, wo_fac)[part - 2][i, c, target, :] = piece.astype(BF16)
                    yield store, y

            def prepare_keys(t, _):
                weight_copy(1, t).wait()
                for store, words in weights(1, t):
                    store(words)

            lax.fori_loop(0, STEPS, prepare_keys, None)
            for t in range(STEPS):
                for copy in wq_copies(t):
                    copy.start()
            for copy in [bx_load] + kv_copies(0) + kv_copies(1):
                copy.start()
            qkv[1:, :, :A_HALO, :] = jnp.zeros((2, 8, A_HALO, 128), BF16)

            def project_rows(part, t, tokens):
                x = ax[word_rows(t), :]
                if part < 2:
                    out = _dot(x, jnp.concatenate([(q_w, k_w)[part][b] for b in range(4)], axis=0))
                    _collect(tokens, 8, 128)(out)
                else:
                    lhs = _factors(x, _LHS)
                    out = _strassen(lambda i: lhs[i], lambda i: _wide(v_fac, i), _collect(tokens, 32, 256))
                if part == 0:
                    out = out * (A_DH ** -0.5 * LOG2E)
                for c, y in enumerate(_chunks(out)):
                    qkv[part, c, pl.ds(pl.multiple_of(t * ROWS + A_HALO, A_HALO), ROWS), :] = y.astype(BF16)

            def keys(t, _):
                for copy in (x_copy(t), weight_copy(0, t), weight_copy(2, t)):
                    copy.wait()
                tokens = []
                project_rows(1, t, tokens)
                _store_spread([*weights(0, t), *weights(2, t)], tokens, _keep(t))

            lax.fori_loop(0, STEPS, keys, None)
            for copy in later_loads:
                copy.wait()

            def queries_values(t, _):
                for copy in wq_copies(t):
                    copy.wait()
                tokens = []
                project_rows(0, t, tokens)
                project_rows(2, t, tokens)
                jobs = list(weights(3, t))
                per_chunk = STEPS // (S // CHUNK)
                n = CHUNK // 8 // per_chunk
                chunk, start = t // per_chunk, pl.multiple_of((t % per_chunk) * n, n)
                words = _slab(lambda row, m: cc[pl.ds(pl.multiple_of(chunk * (CHUNK // 2) + row, m), m), :],
                              CHUNK // 2, start, n)
                for i, y in enumerate(_factors(words, _LHS)):
                    def store(val, i=i):
                        c_fac[chunk, i, pl.ds(pl.multiple_of(2 * start, 2 * n), 2 * n), :] = val.astype(BF16)
                    jobs.append((store, y))
                for piece in range(0, DM // 8, 16):
                    first = pl.multiple_of((t & 1) * (DM // 8) + piece, 16)
                    w = jnp.concatenate([jnp.concatenate(
                        [y for b in range(4) for y in _unpack(wq_raw[t, b, quarter, piece:piece + 16, :])], axis=1)
                        for quarter in range(4)], axis=0)
                    for i, y in enumerate(_factors(w, _RHS)):
                        for e, head in enumerate(_chunks(y)):
                            def store(val, i=i, slot=(t >> 1) * 2 + e, first=first):
                                wq_fac[i, slot, pl.ds(first, 16), :] = val.astype(BF16)
                            jobs.append((store, head))
                _store_spread(jobs, tokens, _keep(t))

            lax.fori_loop(0, STEPS, queries_values, None)

        pl.run_scoped(
            project_a,
            pltpu.VMEM((S // 2, DM), U32), pltpu.VMEM((4, 4, DM // 8, DM), U32), pltpu.VMEM((S // 2, DC), U32),
            pltpu.VMEM((4, DM // 8, DM), U32), pltpu.VMEM((4, DM // 8, DM), U32),
            pltpu.VMEM((PRODUCTS, DM // 512, DM // 4, 128), BF16), pltpu.VMEM((STEPS, 4, 4, DM // 8, D), U32),
            pltpu.SemaphoreType.DMA((5 * STEPS + 2,)))
        for copy in [bx_load] + kv_copies(0):
            copy.wait()

        def project_b(kv32):
            def window_attention(t, tokens):
                first = pl.multiple_of(t * ROWS, ROWS)
                for part in (1, 2):
                    for c in range(8):
                        kv32[part - 1, c] = qkv[part, c, pl.ds(first, A_HALO + ROWS), :].astype(F32)
                lane = lax.broadcasted_iota(jnp.int32, (8, 128), 1)
                sublane = lax.broadcasted_iota(jnp.int32, (8, 128), 0)
                keep = _keep(t)
                groups = ROWS // 8
                period = (len(tokens) / 2.5 - 32) / (groups + 1)

                def at(y, when):
                    return _after(y, tokens[min(int(when * 2.5), len(tokens) - 1)], keep)

                q = []
                for r in range(0, ROWS, 16):
                    both = [qkv[0, c, pl.ds(first + A_HALO + r, 16), :].astype(F32) for c in range(8)]
                    q += [[y[:8] for y in both], [y[8:] for y in both]]

                logits = [[None] * A_WINDOW for _ in range(groups)]
                for g in range(-1, groups):
                    r = A_HALO + 8 * g
                    k = [[kv32[0, c, r - n:r - n + 8, :] for n in (0, 2, 4, 6)] for c in range(8)]
                    for w in range(A_WINDOW):
                        if 0 <= g + w // 4 < groups:
                            logits[g + w // 4][w] = at(_sum([q[g + w // 4][c] * k[c][w % 4] for c in range(8)]),
                                                       (g + 1) * period + 2 * (w % 4) + w // 4)
                p = []
                for g in range(groups):
                    t0 = (g + 1) * period
                    x = logits[g]
                    for bit, lag in ((1, 6), (2, 12)):
                        x = [at(y + jnp.where((lane & bit) != 0, pltpu.roll(y, bit, 1), pltpu.roll(y, 128 - bit, 1)),
                                t0 + lag + (w + 4) % 8) for w, y in enumerate(x)]
                    x = [jnp.where(sublane + first + 8 * g >= 2 * w, y, MASKED) if 8 * g < 2 * w else y
                         for w, y in enumerate(x)]
                    top = x[0]
                    for y in x[1:]:
                        top = jnp.maximum(top, y)
                    x = [jnp.exp2(y - top) for y in x]
                    total = _sum(x)
                    inv = pl.reciprocal(total, approx=True)
                    inv = at(inv * (2.0 - total * inv), t0 + 21)
                    p.append([y * inv for y in x])
                out = [[None] * 8 for _ in range(groups)]
                for g in range(-1, groups):
                    r = A_HALO + 8 * g
                    for c in range(8):
                        before, now = kv32[1, c, r - 8:r, :], kv32[1, c, r:r + 8, :]
                        v = [now] + [pltpu.roll(jnp.where(sublane >= 8 - n, before, now), n, 0) for n in (2, 4, 6)]
                        when = (g + 2) * period + 12 + c
                        if g >= 0:
                            out[g][c] = at(out[g][c] + _sum([p[g][w] * v[w] for w in range(4)]), when)
                        if g + 1 < groups:
                            out[g + 1][c] = at(_sum([p[g + 1][4 + w] * v[w] for w in range(4)]), when)
                    if g > 0 and g % 2:
                        words = _head_shuffle([pltpu.bitcast(jnp.concatenate(both, axis=0).astype(BF16), U32)
                                               for both in zip(out[g - 1], out[g])], inverse=True)
                        rows = pl.ds(pl.multiple_of(first // 2 + 4 * (g - 1), 8), 8)
                        for c, y in enumerate(_chunks(words)):
                            mixed[rows, 128 * c:128 * (c + 1)] = at(y, (g + 2) * period + 24 + c)

            def queries(t, _):
                tokens = []
                lhs = _factors(bx[word_rows(t), :], _LHS)
                q = _strassen(lambda i: lhs[i], lambda i: _wide(wq_fac, i), _collect(tokens, 8, 256))
                for h, y in enumerate(_chunks(q * (D ** -0.5 * LOG2E))):
                    ctx[h, pl.ds(pl.multiple_of(t * ROWS, ROWS), ROWS), :] = y.astype(BF16)
                window_attention(t, tokens)
                _store_spread(list(kv_factors(0, [pl.multiple_of(t * 16, 16)])), tokens, _keep(t))

            lax.fori_loop(0, STEPS, queries, None)

        pl.run_scoped(project_b, pltpu.VMEM((2, 8, A_HALO + ROWS, 128), F32))

    pl.run_scoped(project, pltpu.VMEM((S // 2, DM), U32), pltpu.VMEM((3, 8, A_HALO + S, 128), BF16),
                  pltpu.VMEM((PRODUCTS, H // 4, DM // 4, D), BF16), pltpu.SemaphoreType.DMA)

    def attend(wob, wob_fac, result, sem):
        per_pair = D >> O_LEVELS

        def wob_copy(j):
            rows = pl.ds(pl.multiple_of(j * per_pair, per_pair), per_pair)
            return pltpu.make_async_copy(wob_hbm.bitcast(U32).at[:, rows, :], wob.at[j & 1], sem.at[j & 1])

        wob_copy(0).start()

        def head_pair(j, _):
            @pl.when(j + 1 < H // 2)
            def _():
                wob_copy(j + 1).start()
                for copy in kv_copies(j + 1):
                    copy.wait()

            @pl.when(j + 2 < H // 2)
            def _():
                for copy in kv_copies(j + 2):
                    copy.start()

            wob_copy(j).wait()
            below = (lax.broadcasted_iota(jnp.int32, (TILE, TILE), 1)
                     <= lax.broadcasted_iota(jnp.int32, (TILE, TILE), 0))
            keep = _keep(j)
            ks, vs, scores, results, stored = {}, {}, {}, {}, []

            early = []
            for piece in range(0, per_pair, 8):
                start = pl.multiple_of(j * per_pair + piece, 8)
                words = jnp.concatenate([wob[j & 1, b, piece:piece + 8, :] for b in range(2 ** O_LEVELS)], axis=0)
                for i, y in enumerate(_factors(words, _RHS, O_LEVELS)):
                    def store(val, i=i, start=start):
                        wob_fac[i, pl.ds(pl.multiple_of(2 * start, 16), 16), :] = val.astype(BF16)
                    early.append((store, y))
            late = list(kv_factors(j + 1, range(0, DC // 4, 16)))

            tokens = []
            for chunk in range(S // CHUNK):
                kv = _strassen(lambda i: c_fac.bitcast(U32)[chunk, i], lambda i: wkv_fac.bitcast(U32)[i],
                               _collect(tokens, 32, 128)).astype(BF16)
                for t in range(CHUNK // TILE):
                    k0, k1, v0, v1 = _chunks(kv[t * TILE:(t + 1) * TILE])
                    i = chunk * (CHUNK // TILE) + t
                    ks[0, i], ks[1, i], vs[0, i], vs[1, i] = k0, k1, v0, v1
            _store_spread(early[:len(early) * 7 // 10], tokens[:len(tokens) * 9 // 10], keep)
            late += early[len(early) * 7 // 10:]
            tokens = []

            def score(e, i):
                q = ctx.bitcast(U32)[2 * j + e, i * TILE // 2:(i + 1) * TILE // 2, :]
                while stored:
                    e0, i0 = stored.pop()
                    token = ctx.bitcast(U32)[2 * j + e0 + (j >> 8), i0 * TILE // 2:i0 * TILE // 2 + 8, :]
                    q = jnp.concatenate([_after(q[:8], token, keep), q[8:]], axis=0)
                s = lax.dot_general(pltpu.bitcast(q, BF16),
                                    jnp.concatenate([ks[e, t] for t in range(i + 1)], axis=0),
                                    NT_DIMS, preferred_element_type=F32)
                _collect(tokens, 16, 512)(s)
                diagonal = jnp.where(below, s[:, i * TILE:], MASKED)
                s = jnp.concatenate([s[:, :i * TILE], diagonal], axis=1) if i else diagonal
                scores[e, i] = s, jnp.max(s, axis=1, keepdims=True)

            def context(e, i):
                s, top = scores.pop((e, i))
                p, total = _chunks(jnp.exp2(s - top)), None
                for t in range(0, i + 1, 2):
                    last = min(t + 1, i)
                    total = _sum(p[t:t + 2]) if total is None else total + _sum(p[t:t + 2])
                    p[last] = jnp.concatenate(
                        [_after(p[last][r:r + 8], total[r:r + 8], keep) if r % 32 == 24 else p[last][r:r + 8]
                         for r in range(0, TILE, 8)], axis=0)
                total = jnp.sum(total, axis=1, keepdims=True)
                o = _dot(jnp.concatenate(p, axis=1).astype(BF16),
                         jnp.concatenate([vs[e, t] for t in range(i + 1)], axis=0))
                inv = pl.reciprocal(total, approx=True)
                results[e, i] = (o * (inv * (2.0 - total * inv))).astype(BF16)

            def store_tile(e, i):
                ctx[2 * j + e, i * TILE:(i + 1) * TILE, :] = results.pop((e, i))
                stored.append((e, i))

            for name, tile in _attention_order(S // TILE):
                {"scores": score, "context": context, "store": store_tile}[name](*tile)
            _store_spread(late, tokens[len(tokens) // 10:len(tokens) * 8 // 10], keep)

        lax.fori_loop(0, H // 2, head_pair, None)

        def out_copy(t, side):
            rows = pl.ds(pl.multiple_of(t * ROWS, ROWS), ROWS)
            return pltpu.make_async_copy(result.at[side, t & 1], out_hbm.at[rows, pl.ds(side * DM, DM)],
                                         out_sem.at[2 * side + (t & 1)])

        def outputs(t, _):
            @pl.when(t >= 2)
            def _():
                out_copy(t - 2, 0).wait()
                out_copy(t - 2, 1).wait()

            lhs_b = []
            for g in range(7):
                rows = word_rows(t + (t >> (8 + g)))
                words = jnp.concatenate([ctx.bitcast(U32)[h, rows, :] for h in range(H)], axis=1)
                lhs_b += _factors(words, _LHS, O_LEVELS, g)
            result[1, t & 1] = _strassen(lambda i: lhs_b[i], lambda i: wob_fac.bitcast(U32)[i],
                                         levels=O_LEVELS).astype(BF16)
            lhs_a = _factors(mixed[word_rows(t), :], _LHS)
            products = []

            def send_b(prod):
                products.append(prod)
                if len(products) == 30:
                    out_copy(t, 1).start()

            result[0, t & 1] = _strassen(lambda i: lhs_a[i], lambda i: _wide(wo_fac, i), send_b).astype(BF16)
            out_copy(t, 0).start()

        lax.fori_loop(0, STEPS, outputs, None)
        for t in (STEPS - 2, STEPS - 1):
            out_copy(t, 0).wait()
            out_copy(t, 1).wait()

    pl.run_scoped(
        attend,
        pltpu.VMEM((2, 2 ** O_LEVELS, D >> O_LEVELS, DM), U32),
        pltpu.VMEM((7 ** O_LEVELS, H * D >> O_LEVELS, DM >> O_LEVELS), BF16),
        pltpu.VMEM((2, 2, ROWS, DM), BF16), pltpu.SemaphoreType.DMA((2,)))


@jax.jit
def pallas_concat_heads__sliding_local_dilated__compressed_kv_cla__prompt_kernel(
    A_x: jax.Array,
    A_wqkv: jax.Array,
    A_wo: jax.Array,
    B_x: jax.Array,
    B_c_kv: jax.Array,
    B_w_q: jax.Array,
    B_w_uk: jax.Array,
    B_w_uv: jax.Array,
    B_w_o: jax.Array,
):
    assert A_x.shape == B_x.shape == (1, S, DM) and B_c_kv.shape == (1, S, DC)
    assert B_w_q.shape == (DM, H, D) and B_w_uk.shape == B_w_uv.shape == (DC, H, D)
    out = pl.pallas_call(
        _kernel,
        out_shape=jax.ShapeDtypeStruct((S, 2 * DM), BF16),
        in_specs=[pl.BlockSpec(memory_space=pl.ANY)] * 9,
        out_specs=pl.BlockSpec(memory_space=pl.ANY),
        scratch_shapes=[
            pltpu.VMEM((2, 2, DC, D), U32),
            pltpu.VMEM((S // CHUNK, PRODUCTS, CHUNK // 4, DC // 4), BF16),
            pltpu.VMEM((PRODUCTS, DC // 4, D), BF16), pltpu.VMEM((PRODUCTS, DM // 512, DM // 4, 128), BF16),
            pltpu.VMEM((H, S, D), BF16), pltpu.VMEM((S // 2, DM), U32),
            pltpu.SemaphoreType.DMA((2,)), pltpu.SemaphoreType.DMA((4,)),
        ],
        compiler_params=pltpu.CompilerParams(vmem_limit_bytes=120 * 1024 * 1024),
        name="concat_heads_attention",
    )(
        A_x.reshape(S, DM), A_wqkv.reshape(4, DM // 4, 3 * DM), A_wo.reshape(4, DM // 4, DM),
        B_x.reshape(S, DM), B_c_kv.reshape(S, DC), B_w_q.reshape(4, DM // 4, H // 2, 2, D),
        B_w_uk.reshape(DC, H // 2, 2, D), B_w_uv.reshape(DC, H // 2, 2, D),
        B_w_o.reshape(2 ** O_LEVELS, H * D >> O_LEVELS, DM),
    )
    return out.reshape(1, S, 2 * DM)
```

```python
import math

import jax
import jax.numpy as jnp
from jax import lax
import jax.experimental.pallas as pl
import jax.experimental.pallas.tpu as pltpu

F32, BF16, U32 = jnp.float32, jnp.bfloat16, jnp.uint32
LOG2E = math.log2(math.e)
NT_DIMS = (((1,), (1,)), ((), ()))
MASKED = -1e30

S, DM = 2048, 1024
A_DH, A_WINDOW = 32, 8
A_HALO = 16
H, D, DC = 32, 128, 512
ROWS = 256
STEPS = S // ROWS
CHUNK = 1024
TILE = 128
LEVELS = 2
PRODUCTS = 7 ** LEVELS
O_LEVELS = 3


def _unpack(words):
    return pltpu.bitcast(words << 16, F32), pltpu.bitcast(words & jnp.uint32(0xFFFF0000), F32)


def _chunks(x):
    return [x[:, c:c + 128] for c in range(0, x.shape[1], 128)]


_LHS = ((0, 3, 1), (2, 3, 1), (0, None, 0), (3, None, 0), (0, 1, 1), (2, 0, -1), (1, 3, -1))
_RHS = ((0, 3, 1), (0, None, 0), (1, 3, -1), (2, 0, -1), (3, None, 0), (0, 1, 1), (2, 3, 1))


def _quadrants(x):
    m, n = x.shape[0] // 2, x.shape[1] // 2
    return x[:m, :n], x[:m, n:], x[m:, :n], x[m:, n:]


def _factors(x, recipe, levels=LEVELS, first=None):
    def split(wide, plain, levels, rows):
        if levels == 0:
            return [wide if plain is None else plain]
        quads, out = _quadrants(wide), []
        for a, b, sign in rows:
            if b is None:
                out += split(quads[a], None if plain is None else _quadrants(plain)[a], levels - 1, recipe)
            else:
                out += split(quads[a] + quads[b] if sign > 0 else quads[a] - quads[b], None, levels - 1, recipe)
        return out

    if x.dtype == U32:
        x = pltpu.bitcast(x, BF16)
    return split(x.astype(F32), x, levels, recipe if first is None else [recipe[first]])


def _dot(a, b):
    a, b = [pltpu.bitcast(y, BF16) if y.dtype == U32 else y.astype(BF16) for y in (a, b)]
    return jnp.dot(a, b, preferred_element_type=F32)


def _strassen(lhs, rhs, watch=None, levels=LEVELS, base=0):
    if levels == 0:
        out = _dot(lhs(base), rhs(base))
        if watch is not None:
            watch(out)
        return out
    step = 7 ** (levels - 1)
    m3, m4, m5, m2, m1, m6, m7 = [_strassen(lhs, rhs, watch, levels - 1, base + i * step)
                                  for i in (2, 3, 4, 1, 0, 5, 6)]
    return jnp.concatenate([jnp.concatenate([m4 - m5 + m1 + m7, m3 + m5], axis=1),
                            jnp.concatenate([m2 + m4, m3 - m2 + m1 + m6], axis=1)], axis=0)


def _wide(fac, i):
    return jnp.concatenate([fac.bitcast(U32)[i, c] for c in range(fac.shape[1])], axis=1)


def _slab(load, total, start, n):
    return jnp.concatenate([load(total // 4 * b + start, n) for b in range(4)], axis=0)


def _keep(step):
    return lax.broadcasted_iota(jnp.int32, (8, 128), 1) + step >= 0


def _after(x, token, keep):
    return jnp.where(keep, x, pltpu.bitcast(token, x.dtype))


def _collect(tokens, row_step, col_step):
    return lambda prod: tokens.extend(prod[r:r + 8, c:c + 128] for c in range(0, prod.shape[1], col_step)
                                      for r in range(0, prod.shape[0], row_step))


def _store_spread(jobs, tokens, keep):
    def height(val):
        return 8 if val.dtype == U32 else 16

    jobs = [(store, val.astype(F32) if val.dtype == BF16 else val) for store, val in jobs]
    total = sum(val.size // (128 * height(val)) for _, val in jobs)
    n = 0
    for store, val in jobs:
        rows = []
        for r in range(0, val.shape[0], height(val)):
            cols = []
            for piece in _chunks(val[r:r + 8]):
                cols.append(_after(piece, tokens[n * len(tokens) // total], keep))
                n += 1
            rows.append(jnp.concatenate(cols, axis=1))
            if height(val) == 16:
                rows.append(val[r + 8:r + 16])
        store(jnp.concatenate(rows, axis=0))


def _head_shuffle(chunks, inverse=False):
    group = (lax.broadcasted_iota(jnp.int32, chunks[0].shape, 1) >> 2) & 7

    def rotate(x, c):
        if c == 0:
            return x
        if inverse:
            return jnp.where(group >= c, pltpu.roll(x, 4 * c, 1), pltpu.roll(x, 96 + 4 * c, 1))
        return jnp.where(group < 8 - c, pltpu.roll(x, 128 - 4 * c, 1), pltpu.roll(x, 32 - 4 * c, 1))

    def exchange(xs):
        xs = [xs[-c % 8] for c in range(8)]
        for bit in (1, 2, 4):
            xs = [jnp.where((group & bit) != 0, xs[(c - bit) % 8], xs[c]) for c in range(8)]
        return xs

    if inverse:
        return jnp.concatenate(exchange([rotate(x, c) for c, x in enumerate(chunks)]), axis=1)
    return jnp.concatenate([rotate(x, c) for c, x in enumerate(exchange(chunks))], axis=1)


def _attention_order(n_tiles, lead=8, hold=3):
    tiles = [(e, i) for i in reversed(range(n_tiles)) for e in range(2)]
    steps, done = [], 0
    for t, tile in enumerate(tiles):
        steps.append(("scores", tile))
        while sum(i + 1 for _, i in tiles[done + 1:t + 1]) >= lead:
            steps.append(("context", tiles[done]))
            if done >= hold:
                steps.append(("store", tiles[done - hold]))
            done += 1
    steps += [("context", tile) for tile in tiles[done:]]
    steps += [("store", tile) for tile in tiles[done - hold:]]
    return steps


def _sum(terms):
    return sum(terms[1:], terms[0])


def _kernel(ax_hbm, wqkv_hbm, wo_hbm, bx_hbm, c_hbm, wq_hbm, wuk_hbm, wuv_hbm, wob_hbm, out_hbm,
            wkv_raw, wob_raw, c_fac, wkv_fac, wo_fac, ctx, mixed, in_sem, out_sem):
    def kv_copies(j):
        return [pltpu.make_async_copy(src.bitcast(U32).at[:, j, 0, :], wkv_raw.at[j & 1, i], in_sem.at[j & 1])
                for i, src in enumerate((wuk_hbm, wuv_hbm))]

    per_pair = D >> O_LEVELS

    def wob_copy(j):
        rows = pl.ds(pl.multiple_of(j * per_pair, per_pair), per_pair)
        return pltpu.make_async_copy(wob_hbm.bitcast(U32).at[:, rows, :], wob_raw.at[j & 1], in_sem.at[2 + (j & 1)])

    def kv_factors(j, starts):
        def load(start, n):
            return jnp.concatenate([y for i in range(2) for y in _unpack(wkv_raw[j & 1, i, pl.ds(start, n), :])],
                                   axis=1)

        for start in starts:
            for i, y in enumerate(_factors(_slab(load, DC, start, 16), _RHS)):
                def store(val, i=i, start=start):
                    wkv_fac[i, pl.ds(start, 16), :] = val.astype(BF16)
                yield store, y

    def word_rows(t):
        return pl.ds(pl.multiple_of(t * (ROWS // 2), ROWS // 2), ROWS // 2)

    def project(bx, qkv, wq_fac, bx_sem):
        bx_load = pltpu.make_async_copy(bx_hbm.bitcast(U32), bx, bx_sem)

        def project_a(ax, w_raw, cc, q_w, k_w, v_fac, wq_raw, sem):
            slab = DM // 8 // STEPS

            def weight_copy(part, t):
                rows = pl.ds(t * slab, slab)
                return pltpu.make_async_copy(wqkv_hbm.bitcast(U32).at[:, rows, pl.ds(part * DM, DM)],
                                             w_raw.at[part, :, rows, :], sem.at[part * STEPS + t])

            def x_copy(t):
                rows = pl.ds(t * (ROWS // 2), ROWS // 2)
                return pltpu.make_async_copy(ax_hbm.bitcast(U32).at[rows], ax.at[rows], sem.at[3 * STEPS + t])

            def wq_copies(t):
                rows = pl.ds((t & 1) * (DM // 8), DM // 8)
                return [pltpu.make_async_copy(wq_hbm.bitcast(U32).at[:, rows, 4 * b + (t >> 1), 0, :],
                                              wq_raw.at[t, b], sem.at[4 * STEPS + t]) for b in range(4)]

            later_loads = [pltpu.make_async_copy(src.bitcast(U32), dst, sem.at[5 * STEPS + i])
                           for i, (src, dst) in enumerate(((wo_hbm, w_raw.at[3]), (c_hbm, cc)))]
            for t in range(STEPS):
                weight_copy(1, t).start()
            for t in range(STEPS):
                for copy in (x_copy(t), weight_copy(0, t), weight_copy(2, t)):
                    copy.start()
            for copy in later_loads:
                copy.start()

            def weights(part, t):
                rows = pl.ds(pl.multiple_of(t * slab, slab), slab)
                quarters = [w_raw[part, b, rows, :] for b in range(4)]
                if part < 3:
                    quarters = [_head_shuffle(_chunks(w)) for w in quarters]
                if part >= 2:
                    quarters = _factors(jnp.concatenate(quarters, axis=0), _RHS)
                for i, y in enumerate(quarters):
                    def store(val, i=i):
                        if part < 2:
                            (q_w, k_w)[part][i, rows, :] = val
                        else:
                            for c, piece in enumerate(_chunks(val)):
                                target = pl.ds(pl.multiple_of(t * 2 * slab, 2 * slab), 2 * slab)
                                (v_fac, wo_fac)[part - 2][i, c, target, :] = piece.astype(BF16)
                    yield store, y

            def prepare_keys(t, _):
                weight_copy(1, t).wait()
                for store, words in weights(1, t):
                    store(words)

            lax.fori_loop(0, STEPS, prepare_keys, None)
            for t in range(STEPS):
                for copy in wq_copies(t):
                    copy.start()
            for copy in [bx_load] + kv_copies(0) + kv_copies(1) + [wob_copy(0)]:
                copy.start()
            qkv[1:, :, :A_HALO, :] = jnp.zeros((2, 8, A_HALO, 128), BF16)

            def project_rows(part, t, tokens):
                x = ax[word_rows(t), :]
                if part < 2:
                    out = _dot(x, jnp.concatenate([(q_w, k_w)[part][b] for b in range(4)], axis=0))
                    _collect(tokens, 8, 128)(out)
                else:
                    lhs = _factors(x, _LHS)
                    out = _strassen(lambda i: lhs[i], lambda i: _wide(v_fac, i), _collect(tokens, 32, 256))
                if part == 0:
                    out = out * (A_DH ** -0.5 * LOG2E)
                for c, y in enumerate(_chunks(out)):
                    qkv[part, c, pl.ds(pl.multiple_of(t * ROWS + A_HALO, A_HALO), ROWS), :] = y.astype(BF16)

            def keys(t, _):
                for copy in (x_copy(t), weight_copy(0, t), weight_copy(2, t)):
                    copy.wait()
                tokens = []
                project_rows(1, t, tokens)
                _store_spread([*weights(0, t), *weights(2, t)], tokens, _keep(t))

            lax.fori_loop(0, STEPS, keys, None)
            for copy in later_loads:
                copy.wait()

            def queries_values(t, _):
                for copy in wq_copies(t):
                    copy.wait()
                tokens = []
                project_rows(0, t, tokens)
                project_rows(2, t, tokens)
                jobs = list(weights(3, t))
                per_chunk = STEPS // (S // CHUNK)
                n = CHUNK // 8 // per_chunk
                chunk, start = t // per_chunk, pl.multiple_of((t % per_chunk) * n, n)
                words = _slab(lambda row, m: cc[pl.ds(pl.multiple_of(chunk * (CHUNK // 2) + row, m), m), :],
                              CHUNK // 2, start, n)
                for i, y in enumerate(_factors(words, _LHS)):
                    def store(val, i=i):
                        c_fac[chunk, i, pl.ds(pl.multiple_of(2 * start, 2 * n), 2 * n), :] = val.astype(BF16)
                    jobs.append((store, y))
                for piece in range(0, DM // 8, 16):
                    first = pl.multiple_of((t & 1) * (DM // 8) + piece, 16)
                    w = jnp.concatenate([jnp.concatenate(
                        [y for b in range(4) for y in _unpack(wq_raw[t, b, quarter, piece:piece + 16, :])], axis=1)
                        for quarter in range(4)], axis=0)
                    for i, y in enumerate(_factors(w * (D ** -0.5 * LOG2E), _RHS)):
                        for e, head in enumerate(_chunks(y)):
                            def store(val, i=i, slot=(t >> 1) * 2 + e, first=first):
                                wq_fac[i, slot, pl.ds(first, 16), :] = val.astype(BF16)
                            jobs.append((store, head))
                _store_spread(jobs, tokens, _keep(t))

            lax.fori_loop(0, STEPS, queries_values, None)

        pl.run_scoped(
            project_a,
            pltpu.VMEM((S // 2, DM), U32), pltpu.VMEM((4, 4, DM // 8, DM), U32), pltpu.VMEM((S // 2, DC), U32),
            pltpu.VMEM((4, DM // 8, DM), U32), pltpu.VMEM((4, DM // 8, DM), U32),
            pltpu.VMEM((PRODUCTS, DM // 512, DM // 4, 128), BF16), pltpu.VMEM((STEPS, 4, 4, DM // 8, D), U32),
            pltpu.SemaphoreType.DMA((5 * STEPS + 2,)))
        for copy in [bx_load] + kv_copies(0):
            copy.wait()

        def project_b(kv32):
            def window_attention(t, tokens):
                first = pl.multiple_of(t * ROWS, ROWS)
                for part in (1, 2):
                    for c in range(8):
                        kv32[part - 1, c] = qkv[part, c, pl.ds(first, A_HALO + ROWS), :].astype(F32)
                lane = lax.broadcasted_iota(jnp.int32, (8, 128), 1)
                sublane = lax.broadcasted_iota(jnp.int32, (8, 128), 0)
                keep = _keep(t)
                groups = ROWS // 8
                period = (len(tokens) / 2.5 - 32) / (groups + 1)

                def at(y, when):
                    return _after(y, tokens[min(int(when * 2.5), len(tokens) - 1)], keep)

                q = []
                for r in range(0, ROWS, 16):
                    both = [qkv[0, c, pl.ds(first + A_HALO + r, 16), :].astype(F32) for c in range(8)]
                    q += [[y[:8] for y in both], [y[8:] for y in both]]

                logits = [[None] * A_WINDOW for _ in range(groups)]
                for g in range(-1, groups):
                    r = A_HALO + 8 * g
                    k = [[kv32[0, c, r - n:r - n + 8, :] for n in (0, 2, 4, 6)] for c in range(8)]
                    for w in range(A_WINDOW):
                        if 0 <= g + w // 4 < groups:
                            logits[g + w // 4][w] = at(_sum([q[g + w // 4][c] * k[c][w % 4] for c in range(8)]),
                                                       (g + 1) * period + 2 * (w % 4) + w // 4)
                p = []
                for g in range(groups):
                    t0 = (g + 1) * period
                    x = logits[g]
                    for bit, lag in ((1, 6), (2, 12)):
                        x = [at(y + jnp.where((lane & bit) != 0, pltpu.roll(y, bit, 1), pltpu.roll(y, 128 - bit, 1)),
                                t0 + lag + (w + 4) % 8) for w, y in enumerate(x)]
                    x = [jnp.where(sublane + first + 8 * g >= 2 * w, y, MASKED) if 8 * g < 2 * w else y
                         for w, y in enumerate(x)]
                    top = x[0]
                    for y in x[1:]:
                        top = jnp.maximum(top, y)
                    x = [jnp.exp2(y - top) for y in x]
                    total = _sum(x)
                    inv = pl.reciprocal(total, approx=True)
                    inv = at(inv * (2.0 - total * inv), t0 + 21)
                    p.append([y * inv for y in x])
                out = [[None] * 8 for _ in range(groups)]
                for g in range(-1, groups):
                    r = A_HALO + 8 * g
                    for c in range(8):
                        before, now = kv32[1, c, r - 8:r, :], kv32[1, c, r:r + 8, :]
                        v = [now] + [pltpu.roll(jnp.where(sublane >= 8 - n, before, now), n, 0) for n in (2, 4, 6)]
                        when = (g + 2) * period + 12 + c
                        if g >= 0:
                            out[g][c] = at(out[g][c] + _sum([p[g][w] * v[w] for w in range(4)]), when)
                        if g + 1 < groups:
                            out[g + 1][c] = at(_sum([p[g + 1][4 + w] * v[w] for w in range(4)]), when)
                    if g > 0 and g % 2:
                        words = _head_shuffle([pltpu.bitcast(jnp.concatenate(both, axis=0).astype(BF16), U32)
                                               for both in zip(out[g - 1], out[g])], inverse=True)
                        rows = pl.ds(pl.multiple_of(first // 2 + 4 * (g - 1), 8), 8)
                        for c, y in enumerate(_chunks(words)):
                            mixed[rows, 128 * c:128 * (c + 1)] = at(y, (g + 2) * period + 24 + c)

            def queries(t, _):
                tokens = []
                lhs = _factors(bx[word_rows(t), :], _LHS)
                q = _strassen(lambda i: lhs[i], lambda i: _wide(wq_fac, i), _collect(tokens, 8, 256))
                for h, y in enumerate(_chunks(q)):
                    ctx[h, pl.ds(pl.multiple_of(t * ROWS, ROWS), ROWS), :] = y.astype(BF16)
                window_attention(t, tokens)
                _store_spread(list(kv_factors(0, [pl.multiple_of(t * 16, 16)])), tokens, _keep(t))

            lax.fori_loop(0, STEPS, queries, None)

        pl.run_scoped(project_b, pltpu.VMEM((2, 8, A_HALO + ROWS, 128), F32))

    pl.run_scoped(project, pltpu.VMEM((S // 2, DM), U32), pltpu.VMEM((3, 8, A_HALO + S, 128), BF16),
                  pltpu.VMEM((PRODUCTS, H // 4, DM // 4, D), BF16), pltpu.SemaphoreType.DMA)

    def attend(wob_fac, kv, result):
        def head_pair(j, _):
            @pl.when(j + 1 < H // 2)
            def _():
                wob_copy(j + 1).start()
                for copy in kv_copies(j + 1):
                    copy.wait()

            @pl.when(j + 2 < H // 2)
            def _():
                for copy in kv_copies(j + 2):
                    copy.start()

            wob_copy(j).wait()
            below = (lax.broadcasted_iota(jnp.int32, (TILE, TILE), 1)
                     <= lax.broadcasted_iota(jnp.int32, (TILE, TILE), 0))
            keep = _keep(j)
            scores, results, stored = {}, {}, []

            early = []
            for piece in range(0, per_pair, 8):
                start = pl.multiple_of(j * per_pair + piece, 8)
                words = jnp.concatenate([wob_raw[j & 1, b, piece:piece + 8, :] for b in range(2 ** O_LEVELS)],
                                        axis=0)
                for i, y in enumerate(_factors(words, _RHS, O_LEVELS)):
                    def store(val, i=i, start=start):
                        wob_fac[i, pl.ds(pl.multiple_of(2 * start, 16), 16), :] = val.astype(BF16)
                    early.append((store, y))
            late = list(kv_factors(j + 1, range(0, DC // 4, 16)))

            tokens = []
            for chunk in range(S // CHUNK):
                out = _strassen(lambda i: c_fac.bitcast(U32)[chunk, i], lambda i: wkv_fac.bitcast(U32)[i],
                                _collect(tokens, 16, 128))
                for n, y in enumerate(_chunks(out)):
                    kv[n, chunk * CHUNK:(chunk + 1) * CHUNK, :] = y.astype(BF16)
            _store_spread(early[:len(early) * 7 // 10], tokens[:len(tokens) * 8 // 10], keep)
            late = early[len(early) * 7 // 10:] + late
            tokens = []

            def score(e, i):
                q = ctx.bitcast(U32)[2 * j + e, i * TILE // 2:(i + 1) * TILE // 2, :]
                while stored:
                    e0, i0 = stored.pop()
                    token = ctx.bitcast(U32)[2 * j + e0 + (j >> 8), i0 * TILE // 2:i0 * TILE // 2 + 8, :]
                    q = jnp.concatenate([_after(q[:8], token, keep), q[8:]], axis=0)
                k = kv.bitcast(U32)[e, :(i + 1) * TILE // 2, :]
                s = lax.dot_general(pltpu.bitcast(q, BF16), pltpu.bitcast(k, BF16), NT_DIMS,
                                    preferred_element_type=F32)
                _collect(tokens, 8, 512)(s)
                diagonal = jnp.where(below, s[:, i * TILE:], MASKED)
                s = jnp.concatenate([s[:, :i * TILE], diagonal], axis=1) if i else diagonal
                scores[e, i] = s, jnp.max(s, axis=1, keepdims=True)

            def context(e, i):
                s, top = scores.pop((e, i))
                p, total = _chunks(jnp.exp2(s - top)), None
                for t in range(0, i + 1, 2):
                    last = min(t + 1, i)
                    total = _sum(p[t:t + 2]) if total is None else total + _sum(p[t:t + 2])
                    p[last] = jnp.concatenate(
                        [_after(p[last][r:r + 8], total[r:r + 8], keep) if r % 16 else p[last][r:r + 8]
                         for r in range(0, TILE, 8)], axis=0)
                total = jnp.sum(total, axis=1, keepdims=True)
                o = _dot(jnp.concatenate(p, axis=1), kv.bitcast(U32)[2 + e, :(i + 1) * TILE // 2, :])
                inv = pl.reciprocal(total, approx=True)
                results[e, i] = (o * (inv * (2.0 - total * inv))).astype(BF16)

            def store_tile(e, i):
                ctx[2 * j + e, i * TILE:(i + 1) * TILE, :] = results.pop((e, i))
                stored.append((e, i))

            for name, tile in _attention_order(S // TILE):
                {"scores": score, "context": context, "store": store_tile}[name](*tile)
            _store_spread(late, tokens[len(tokens) // 10:len(tokens) * 19 // 20], keep)

        lax.fori_loop(0, H // 2, head_pair, None)

        def out_copy(t, side):
            rows = pl.ds(pl.multiple_of(t * ROWS, ROWS), ROWS)
            return pltpu.make_async_copy(result.at[side, t & 1], out_hbm.at[rows, pl.ds(side * DM, DM)],
                                         out_sem.at[2 * side + (t & 1)])

        def outputs(t, _):
            @pl.when(t >= 2)
            def _():
                out_copy(t - 2, 0).wait()
                out_copy(t - 2, 1).wait()

            lhs_b = []
            for g in range(7):
                rows = word_rows(t + (t >> (8 + g)))
                words = jnp.concatenate([ctx.bitcast(U32)[h, rows, :] for h in range(H)], axis=1)
                lhs_b += _factors(words, _LHS, O_LEVELS, g)
            result[1, t & 1] = _strassen(lambda i: lhs_b[i], lambda i: wob_fac.bitcast(U32)[i],
                                         levels=O_LEVELS).astype(BF16)
            lhs_a = _factors(mixed[word_rows(t), :], _LHS)
            products = []

            def send_b(prod):
                products.append(prod)
                if len(products) == 30:
                    out_copy(t, 1).start()

            result[0, t & 1] = _strassen(lambda i: lhs_a[i], lambda i: _wide(wo_fac, i), send_b).astype(BF16)
            out_copy(t, 0).start()

        lax.fori_loop(0, STEPS, outputs, None)
        for t in (STEPS - 2, STEPS - 1):
            out_copy(t, 0).wait()
            out_copy(t, 1).wait()

    pl.run_scoped(
        attend,
        pltpu.VMEM((7 ** O_LEVELS, H * D >> O_LEVELS, DM >> O_LEVELS), BF16),
        pltpu.VMEM((4, S, D), BF16), pltpu.VMEM((2, 2, ROWS, DM), BF16))


@jax.jit
def pallas_concat_heads__sliding_local_dilated__compressed_kv_cla__prompt_kernel(
    A_x: jax.Array,
    A_wqkv: jax.Array,
    A_wo: jax.Array,
    B_x: jax.Array,
    B_c_kv: jax.Array,
    B_w_q: jax.Array,
    B_w_uk: jax.Array,
    B_w_uv: jax.Array,
    B_w_o: jax.Array,
):
    assert A_x.shape == B_x.shape == (1, S, DM) and B_c_kv.shape == (1, S, DC)
    assert B_w_q.shape == (DM, H, D) and B_w_uk.shape == B_w_uv.shape == (DC, H, D)
    out = pl.pallas_call(
        _kernel,
        out_shape=jax.ShapeDtypeStruct((S, 2 * DM), BF16),
        in_specs=[pl.BlockSpec(memory_space=pl.ANY)] * 9,
        out_specs=pl.BlockSpec(memory_space=pl.ANY),
        scratch_shapes=[
            pltpu.VMEM((2, 2, DC, D), U32), pltpu.VMEM((2, 2 ** O_LEVELS, D >> O_LEVELS, DM), U32),
            pltpu.VMEM((S // CHUNK, PRODUCTS, CHUNK // 4, DC // 4), BF16),
            pltpu.VMEM((PRODUCTS, DC // 4, D), BF16), pltpu.VMEM((PRODUCTS, DM // 512, DM // 4, 128), BF16),
            pltpu.VMEM((H, S, D), BF16), pltpu.VMEM((S // 2, DM), U32),
            pltpu.SemaphoreType.DMA((4,)), pltpu.SemaphoreType.DMA((4,)),
        ],
        compiler_params=pltpu.CompilerParams(vmem_limit_bytes=120 * 1024 * 1024),
        name="concat_heads_attention",
    )(
        A_x.reshape(S, DM), A_wqkv.reshape(4, DM // 4, 3 * DM), A_wo.reshape(4, DM // 4, DM),
        B_x.reshape(S, DM), B_c_kv.reshape(S, DC), B_w_q.reshape(4, DM // 4, H // 2, 2, D),
        B_w_uk.reshape(DC, H // 2, 2, D), B_w_uv.reshape(DC, H // 2, 2, D),
        B_w_o.reshape(2 ** O_LEVELS, H * D >> O_LEVELS, DM),
    )
    return out.reshape(1, S, 2 * DM)
```

```python
import math

import jax
import jax.numpy as jnp
from jax import lax
import jax.experimental.pallas as pl
import jax.experimental.pallas.tpu as pltpu

F32, BF16, U32 = jnp.float32, jnp.bfloat16, jnp.uint32
LOG2E = math.log2(math.e)
NT_DIMS = (((1,), (1,)), ((), ()))
MASKED = -1e30

S, DM = 2048, 1024
A_DH, A_WINDOW = 32, 8
A_HALO = 16
H, D, DC = 32, 128, 512
ROWS = 256
STEPS = S // ROWS
CHUNK = 1024
TILE = 128
LEVELS = 2
PRODUCTS = 7 ** LEVELS
O_LEVELS = 3


def _unpack(words):
    return pltpu.bitcast(words << 16, F32), pltpu.bitcast(words & jnp.uint32(0xFFFF0000), F32)


def _chunks(x):
    return [x[:, c:c + 128] for c in range(0, x.shape[1], 128)]


_LHS = ((0, 3, 1), (2, 3, 1), (0, None, 0), (3, None, 0), (0, 1, 1), (2, 0, -1), (1, 3, -1))
_RHS = ((0, 3, 1), (0, None, 0), (1, 3, -1), (2, 0, -1), (3, None, 0), (0, 1, 1), (2, 3, 1))


def _quadrants(x):
    m, n = x.shape[0] // 2, x.shape[1] // 2
    return x[:m, :n], x[:m, n:], x[m:, :n], x[m:, n:]


def _factors(x, recipe, levels=LEVELS, first=None):
    def split(wide, plain, levels, rows):
        if levels == 0:
            return [wide if plain is None else plain]
        quads, out = _quadrants(wide), []
        for a, b, sign in rows:
            if b is None:
                out += split(quads[a], None if plain is None else _quadrants(plain)[a], levels - 1, recipe)
            else:
                out += split(quads[a] + quads[b] if sign > 0 else quads[a] - quads[b], None, levels - 1, recipe)
        return out

    if x.dtype == U32:
        x = pltpu.bitcast(x, BF16)
    return split(x.astype(F32), x, levels, recipe if first is None else [recipe[first]])


def _dot(a, b):
    a, b = [pltpu.bitcast(y, BF16) if y.dtype == U32 else y.astype(BF16) for y in (a, b)]
    return jnp.dot(a, b, preferred_element_type=F32)


def _quadrant_sums(product):
    m3, m4, m5 = product(2), product(3), product(4)
    yield 1, m3 + m5
    m2 = product(1)
    yield 2, m2 + m4
    m1, m6 = product(0), product(5)
    yield 3, m3 - m2 + m1 + m6
    yield 0, m4 - m5 + m1 + product(6)


def _strassen(lhs, rhs, watch=None, levels=LEVELS, base=0):
    if levels == 0:
        out = _dot(lhs(base), rhs(base))
        if watch is not None:
            watch(out)
        return out
    step = 7 ** (levels - 1)
    done = dict(_quadrant_sums(lambda i: _strassen(lhs, rhs, watch, levels - 1, base + i * step)))
    return jnp.concatenate([jnp.concatenate([done[0], done[1]], axis=1),
                            jnp.concatenate([done[2], done[3]], axis=1)], axis=0)


def _wide(fac, i):
    return jnp.concatenate([fac.bitcast(U32)[i, c] for c in range(fac.shape[1])], axis=1)


def _slab(load, total, start, n):
    return jnp.concatenate([load(total // 4 * b + start, n) for b in range(4)], axis=0)


def _keep(step):
    return lax.broadcasted_iota(jnp.int32, (8, 128), 1) + step >= 0


def _after(x, token, keep):
    return jnp.where(keep, x, pltpu.bitcast(token, x.dtype))


def _collect(tokens, row_step, col_step):
    return lambda prod: tokens.extend(prod[r:r + 8, c:c + 128] for c in range(0, prod.shape[1], col_step)
                                      for r in range(0, prod.shape[0], row_step))


def _store_spread(jobs, tokens, keep):
    def height(val):
        return 8 if val.dtype == U32 else 16

    jobs = [(store, val.astype(F32) if val.dtype == BF16 else val) for store, val in jobs]
    total = sum(val.size // (128 * height(val)) for _, val in jobs)
    n = 0
    for store, val in jobs:
        rows = []
        for r in range(0, val.shape[0], height(val)):
            cols = []
            for piece in _chunks(val[r:r + 8]):
                cols.append(_after(piece, tokens[n * len(tokens) // total], keep))
                n += 1
            rows.append(jnp.concatenate(cols, axis=1))
            if height(val) == 16:
                rows.append(val[r + 8:r + 16])
        store(jnp.concatenate(rows, axis=0))


def _head_shuffle(chunks, inverse=False):
    group = (lax.broadcasted_iota(jnp.int32, chunks[0].shape, 1) >> 2) & 7

    def rotate(x, c):
        if c == 0:
            return x
        if inverse:
            return jnp.where(group >= c, pltpu.roll(x, 4 * c, 1), pltpu.roll(x, 96 + 4 * c, 1))
        return jnp.where(group < 8 - c, pltpu.roll(x, 128 - 4 * c, 1), pltpu.roll(x, 32 - 4 * c, 1))

    def exchange(xs):
        xs = [xs[-c % 8] for c in range(8)]
        for bit in (1, 2, 4):
            xs = [jnp.where((group & bit) != 0, xs[(c - bit) % 8], xs[c]) for c in range(8)]
        return xs

    if inverse:
        return jnp.concatenate(exchange([rotate(x, c) for c, x in enumerate(chunks)]), axis=1)
    return jnp.concatenate([rotate(x, c) for c, x in enumerate(exchange(chunks))], axis=1)


def _attention_order(n_tiles, lead=8, hold=3):
    tiles = [(e, i) for i in reversed(range(n_tiles)) for e in range(2)]
    steps, done = [], 0
    for t, tile in enumerate(tiles):
        steps.append(("scores", tile))
        while sum(i + 1 for _, i in tiles[done + 1:t + 1]) >= lead:
            steps.append(("context", tiles[done]))
            if done >= hold:
                steps.append(("store", tiles[done - hold]))
            done += 1
    steps += [("context", tile) for tile in tiles[done:]]
    steps += [("store", tile) for tile in tiles[done - hold:]]
    return steps


def _sum(terms):
    return sum(terms[1:], terms[0])


def _kernel(ax_hbm, wqkv_hbm, wo_hbm, bx_hbm, c_hbm, wq_hbm, wuk_hbm, wuv_hbm, wob_hbm, out_hbm,
            wkv_raw, wob_raw, c_fac, wkv_fac, wo_fac, ctx, mixed, in_sem, out_sem):
    def kv_copies(j):
        return [pltpu.make_async_copy(src.bitcast(U32).at[:, j, 0, :], wkv_raw.at[j & 1, i], in_sem.at[j & 1])
                for i, src in enumerate((wuk_hbm, wuv_hbm))]

    per_pair = D >> O_LEVELS

    def wob_copy(j):
        rows = pl.ds(pl.multiple_of(j * per_pair, per_pair), per_pair)
        return pltpu.make_async_copy(wob_hbm.bitcast(U32).at[:, rows, :], wob_raw.at[j & 1], in_sem.at[2 + (j & 1)])

    def kv_factors(j, starts):
        def load(start, n):
            return jnp.concatenate([y for i in range(2) for y in _unpack(wkv_raw[j & 1, i, pl.ds(start, n), :])],
                                   axis=1)

        for start in starts:
            for i, y in enumerate(_factors(_slab(load, DC, start, 16), _RHS)):
                def store(val, i=i, start=start):
                    wkv_fac[i, pl.ds(start, 16), :] = val.astype(BF16)
                yield store, y

    def word_rows(t):
        return pl.ds(pl.multiple_of(t * (ROWS // 2), ROWS // 2), ROWS // 2)

    def project(bx, qkv, wq_fac, bx_sem):
        bx_load = pltpu.make_async_copy(bx_hbm.bitcast(U32), bx, bx_sem)

        def project_a(ax, w_raw, cc, q_w, k_w, v_fac, wq_raw, sem):
            slab = DM // 8 // STEPS

            def weight_copy(part, t):
                rows = pl.ds(t * slab, slab)
                return pltpu.make_async_copy(wqkv_hbm.bitcast(U32).at[:, rows, pl.ds(part * DM, DM)],
                                             w_raw.at[part, :, rows, :], sem.at[part * STEPS + t])

            def x_copy(t):
                rows = pl.ds(t * (ROWS // 2), ROWS // 2)
                return pltpu.make_async_copy(ax_hbm.bitcast(U32).at[rows], ax.at[rows], sem.at[3 * STEPS + t])

            def wq_copies(t):
                rows = pl.ds((t & 1) * (DM // 8), DM // 8)
                return [pltpu.make_async_copy(wq_hbm.bitcast(U32).at[:, rows, 4 * b + (t >> 1), 0, :],
                                              wq_raw.at[t, b], sem.at[4 * STEPS + t]) for b in range(4)]

            later_loads = [pltpu.make_async_copy(src.bitcast(U32), dst, sem.at[5 * STEPS + i])
                           for i, (src, dst) in enumerate(((wo_hbm, w_raw.at[3]), (c_hbm, cc)))]
            for t in range(STEPS):
                weight_copy(1, t).start()
            for t in range(STEPS):
                for copy in (x_copy(t), weight_copy(0, t), weight_copy(2, t)):
                    copy.start()
            for copy in later_loads:
                copy.start()

            def weights(part, t):
                rows = pl.ds(pl.multiple_of(t * slab, slab), slab)
                quarters = [w_raw[part, b, rows, :] for b in range(4)]
                if part < 3:
                    quarters = [_head_shuffle(_chunks(w)) for w in quarters]
                if part >= 2:
                    quarters = _factors(jnp.concatenate(quarters, axis=0), _RHS)
                for i, y in enumerate(quarters):
                    def store(val, i=i):
                        if part < 2:
                            (q_w, k_w)[part][i, rows, :] = val
                        else:
                            for c, piece in enumerate(_chunks(val)):
                                target = pl.ds(pl.multiple_of(t * 2 * slab, 2 * slab), 2 * slab)
                                (v_fac, wo_fac)[part - 2][i, c, target, :] = piece.astype(BF16)
                    yield store, y

            def prepare_keys(t, _):
                weight_copy(1, t).wait()
                for store, words in weights(1, t):
                    store(words)

            lax.fori_loop(0, STEPS, prepare_keys, None)
            for t in range(STEPS):
                for copy in wq_copies(t):
                    copy.start()
            for copy in [bx_load] + kv_copies(0) + kv_copies(1) + [wob_copy(0)]:
                copy.start()
            qkv[1:, :, :A_HALO, :] = jnp.zeros((2, 8, A_HALO, 128), BF16)

            def project_rows(part, t, tokens):
                x = ax[word_rows(t), :]
                if part < 2:
                    out = _dot(x, jnp.concatenate([(q_w, k_w)[part][b] for b in range(4)], axis=0))
                    _collect(tokens, 8, 128)(out)
                else:
                    lhs = _factors(x, _LHS)
                    out = _strassen(lambda i: lhs[i], lambda i: _wide(v_fac, i), _collect(tokens, 32, 256))
                for c, y in enumerate(_chunks(out)):
                    qkv[part, c, pl.ds(pl.multiple_of(t * ROWS + A_HALO, A_HALO), ROWS), :] = y.astype(BF16)

            def keys(t, _):
                for copy in (x_copy(t), weight_copy(0, t), weight_copy(2, t)):
                    copy.wait()
                tokens = []
                project_rows(1, t, tokens)
                _store_spread([*weights(0, t), *weights(2, t)], tokens, _keep(t))

            lax.fori_loop(0, STEPS, keys, None)
            for copy in later_loads:
                copy.wait()

            def queries_values(t, _):
                for copy in wq_copies(t):
                    copy.wait()
                tokens = []
                project_rows(0, t, tokens)
                project_rows(2, t, tokens)
                jobs = list(weights(3, t))
                per_chunk = STEPS // (S // CHUNK)
                n = CHUNK // 8 // per_chunk
                chunk, start = t // per_chunk, pl.multiple_of((t % per_chunk) * n, n)
                words = _slab(lambda row, m: cc[pl.ds(pl.multiple_of(chunk * (CHUNK // 2) + row, m), m), :],
                              CHUNK // 2, start, n)
                for i, y in enumerate(_factors(words, _LHS)):
                    def store(val, i=i):
                        c_fac[chunk, i, pl.ds(pl.multiple_of(2 * start, 2 * n), 2 * n), :] = val.astype(BF16)
                    jobs.append((store, y))
                for piece in range(0, DM // 8, 16):
                    first = pl.multiple_of((t & 1) * (DM // 8) + piece, 16)
                    w = jnp.concatenate([jnp.concatenate(
                        [y for b in range(4) for y in _unpack(wq_raw[t, b, quarter, piece:piece + 16, :])], axis=1)
                        for quarter in range(4)], axis=0)
                    for i, y in enumerate(_factors(w * (D ** -0.5 * LOG2E), _RHS)):
                        for e, head in enumerate(_chunks(y)):
                            def store(val, i=i, slot=(t >> 1) * 2 + e, first=first):
                                wq_fac[i, slot, pl.ds(first, 16), :] = val.astype(BF16)
                            jobs.append((store, head))
                _store_spread(jobs, tokens, _keep(t))

            lax.fori_loop(0, STEPS, queries_values, None)

        pl.run_scoped(
            project_a,
            pltpu.VMEM((S // 2, DM), U32), pltpu.VMEM((4, 4, DM // 8, DM), U32), pltpu.VMEM((S // 2, DC), U32),
            pltpu.VMEM((4, DM // 8, DM), U32), pltpu.VMEM((4, DM // 8, DM), U32),
            pltpu.VMEM((PRODUCTS, DM // 512, DM // 4, 128), BF16), pltpu.VMEM((STEPS, 4, 4, DM // 8, D), U32),
            pltpu.SemaphoreType.DMA((5 * STEPS + 2,)))
        for copy in [bx_load] + kv_copies(0):
            copy.wait()

        def project_b(kv32):
            def window_attention(t, tokens):
                first = pl.multiple_of(t * ROWS, ROWS)
                for part in (1, 2):
                    for c in range(8):
                        kv32[part - 1, c] = qkv[part, c, pl.ds(first, A_HALO + ROWS), :].astype(F32)
                lane = lax.broadcasted_iota(jnp.int32, (8, 128), 1)
                sublane = lax.broadcasted_iota(jnp.int32, (8, 128), 0)
                keep = _keep(t)
                groups = ROWS // 8
                period = (len(tokens) / 2.5 - 32) / (groups + 1)

                def at(y, when):
                    return _after(y, tokens[min(int(when * 2.5), len(tokens) - 1)], keep)

                q = []
                for r in range(0, ROWS, 16):
                    both = [qkv[0, c, pl.ds(first + A_HALO + r, 16), :].astype(F32) for c in range(8)]
                    q += [[y[:8] for y in both], [y[8:] for y in both]]

                logits = [[None] * A_WINDOW for _ in range(groups)]
                for g in range(-1, groups):
                    r = A_HALO + 8 * g
                    k = [[kv32[0, c, r - n:r - n + 8, :] for n in (0, 2, 4, 6)] for c in range(8)]
                    for w in range(A_WINDOW):
                        if 0 <= g + w // 4 < groups:
                            logits[g + w // 4][w] = at(_sum([q[g + w // 4][c] * k[c][w % 4] for c in range(8)]),
                                                       (g + 1) * period + 2 * (w % 4) + w // 4)
                p = []
                for g in range(groups):
                    t0 = (g + 1) * period
                    x = logits[g]
                    for bit, lag in ((1, 6), (2, 12)):
                        x = [at(y + jnp.where((lane & bit) != 0, pltpu.roll(y, bit, 1), pltpu.roll(y, 128 - bit, 1)),
                                t0 + lag + (w + 4) % 8) for w, y in enumerate(x)]
                    x = [jnp.where(sublane + first + 8 * g >= 2 * w, y, MASKED) if 8 * g < 2 * w else y
                         for w, y in enumerate(x)]
                    top = x[0]
                    for y in x[1:]:
                        top = jnp.maximum(top, y)
                    x = [jnp.exp2((y - top) * (A_DH ** -0.5 * LOG2E)) for y in x]
                    total = _sum(x)
                    inv = pl.reciprocal(total, approx=True)
                    inv = at(inv * (2.0 - total * inv), t0 + 23)
                    p.append([y * inv for y in x])
                out = [[None] * 8 for _ in range(groups)]
                for g in range(-1, groups):
                    r = A_HALO + 8 * g
                    for c in range(8):
                        before, now = kv32[1, c, r - 8:r, :], kv32[1, c, r:r + 8, :]
                        v = [now] + [pltpu.roll(jnp.where(sublane >= 8 - n, before, now), n, 0) for n in (2, 4, 6)]
                        when = (g + 2) * period + 12 + c
                        if g >= 0:
                            out[g][c] = at(out[g][c] + _sum([p[g][w] * v[w] for w in range(4)]), when)
                        if g + 1 < groups:
                            out[g + 1][c] = at(_sum([p[g + 1][4 + w] * v[w] for w in range(4)]), when)
                    if g > 0 and g % 2:
                        words = _head_shuffle([pltpu.bitcast(jnp.concatenate(both, axis=0).astype(BF16), U32)
                                               for both in zip(out[g - 1], out[g])], inverse=True)
                        rows = pl.ds(pl.multiple_of(first // 2 + 4 * (g - 1), 8), 8)
                        for c, y in enumerate(_chunks(words)):
                            mixed[rows, 128 * c:128 * (c + 1)] = at(y, (g + 2) * period + 24 + c)

            def queries(t, _):
                tokens = []
                lhs = _factors(bx[word_rows(t), :], _LHS)
                q = _strassen(lambda i: lhs[i], lambda i: _wide(wq_fac, i), _collect(tokens, 8, 256))
                for h, y in enumerate(_chunks(q)):
                    ctx[h, pl.ds(pl.multiple_of(t * ROWS, ROWS), ROWS), :] = y.astype(BF16)
                window_attention(t, tokens)
                _store_spread(list(kv_factors(0, [pl.multiple_of(t * 16, 16)])), tokens, _keep(t))

            lax.fori_loop(0, STEPS, queries, None)

        pl.run_scoped(project_b, pltpu.VMEM((2, 8, A_HALO + ROWS, 128), F32))

    pl.run_scoped(project, pltpu.VMEM((S // 2, DM), U32), pltpu.VMEM((3, 8, A_HALO + S, 128), BF16),
                  pltpu.VMEM((PRODUCTS, H // 4, DM // 4, D), BF16), pltpu.SemaphoreType.DMA)

    def attend(wob_fac, kv, result):
        def head_pair(j, _):
            @pl.when(j + 1 < H // 2)
            def _():
                wob_copy(j + 1).start()
                for copy in kv_copies(j + 1):
                    copy.wait()

            @pl.when(j + 2 < H // 2)
            def _():
                for copy in kv_copies(j + 2):
                    copy.start()

            wob_copy(j).wait()
            below = (lax.broadcasted_iota(jnp.int32, (TILE, TILE), 1)
                     <= lax.broadcasted_iota(jnp.int32, (TILE, TILE), 0))
            keep = _keep(j)
            scores, results, stored = {}, {}, []

            early = []
            for piece in range(0, per_pair, 8):
                start = pl.multiple_of(j * per_pair + piece, 8)
                words = jnp.concatenate([wob_raw[j & 1, b, piece:piece + 8, :] for b in range(2 ** O_LEVELS)],
                                        axis=0)
                for i, y in enumerate(_factors(words, _RHS, O_LEVELS)):
                    def store(val, i=i, start=start):
                        wob_fac[i, pl.ds(pl.multiple_of(2 * start, 16), 16), :] = val.astype(BF16)
                    early.append((store, y))
            late = list(kv_factors(j + 1, range(0, DC // 4, 16)))

            tokens = []
            for chunk in range(S // CHUNK):
                out = _strassen(lambda i: c_fac.bitcast(U32)[chunk, i], lambda i: wkv_fac.bitcast(U32)[i],
                                _collect(tokens, 16, 128))
                for n, y in enumerate(_chunks(out)):
                    kv[n, chunk * CHUNK:(chunk + 1) * CHUNK, :] = y.astype(BF16)
            _store_spread(early[:len(early) * 7 // 10], tokens[:len(tokens) * 8 // 10], keep)
            late = early[len(early) * 7 // 10:] + late
            tokens = []

            def score(e, i):
                q = ctx.bitcast(U32)[2 * j + e, i * TILE // 2:(i + 1) * TILE // 2, :]
                while stored:
                    e0, i0 = stored.pop()
                    token = ctx.bitcast(U32)[2 * j + e0 + (j >> 8), i0 * TILE // 2:i0 * TILE // 2 + 8, :]
                    q = jnp.concatenate([_after(q[:8], token, keep), q[8:]], axis=0)
                k = kv.bitcast(U32)[e, :(i + 1) * TILE // 2, :]
                s = lax.dot_general(pltpu.bitcast(q, BF16), pltpu.bitcast(k, BF16), NT_DIMS,
                                    preferred_element_type=F32)
                _collect(tokens, 8, 512)(s)
                diagonal = jnp.where(below, s[:, i * TILE:], MASKED)
                s = jnp.concatenate([s[:, :i * TILE], diagonal], axis=1) if i else diagonal
                scores[e, i] = s, jnp.max(s, axis=1, keepdims=True)

            def context(e, i):
                s, top = scores.pop((e, i))
                p, total = _chunks(jnp.exp2(s - top)), None
                for t in range(0, i + 1, 2):
                    last = min(t + 1, i)
                    total = _sum(p[t:t + 2]) if total is None else total + _sum(p[t:t + 2])
                    p[last] = jnp.concatenate(
                        [_after(p[last][r:r + 8], total[r:r + 8], keep) if r % 16 else p[last][r:r + 8]
                         for r in range(0, TILE, 8)], axis=0)
                total = jnp.sum(total, axis=1, keepdims=True)
                o = _dot(jnp.concatenate(p, axis=1), kv.bitcast(U32)[2 + e, :(i + 1) * TILE // 2, :])
                inv = pl.reciprocal(total, approx=True)
                results[e, i] = (o * (inv * (2.0 - total * inv))).astype(BF16)

            def store_tile(e, i):
                ctx[2 * j + e, i * TILE:(i + 1) * TILE, :] = results.pop((e, i))
                stored.append((e, i))

            for name, tile in _attention_order(S // TILE):
                {"scores": score, "context": context, "store": store_tile}[name](*tile)
            _store_spread(late, tokens[len(tokens) // 10:len(tokens) * 19 // 20], keep)

        lax.fori_loop(0, H // 2, head_pair, None)

        def out_copies(t):
            def copy(side, row, col, rows, cols):
                return pltpu.make_async_copy(
                    result.at[side, t & 1, pl.ds(row, rows), pl.ds(col, cols)],
                    out_hbm.at[pl.ds(pl.multiple_of(t * ROWS + row, rows), rows), pl.ds(side * DM + col, cols)],
                    out_sem.at[t & 1])

            return [copy(1, 0, 0, ROWS, DM)] + [copy(0, n // 2 * (ROWS // 2), n % 2 * (DM // 2), ROWS // 2, DM // 2)
                                                for n in range(4)]

        def outputs(t, _):
            @pl.when(t >= 2)
            def _():
                for copy in out_copies(t - 2):
                    copy.wait()

            lhs_b = []
            for g in range(7):
                rows = word_rows(t + (t >> (8 + g)))
                words = jnp.concatenate([ctx.bitcast(U32)[h, rows, :] for h in range(H)], axis=1)
                lhs_b += _factors(words, _LHS, O_LEVELS, g)
            result[1, t & 1] = _strassen(lambda i: lhs_b[i], lambda i: wob_fac.bitcast(U32)[i],
                                         levels=O_LEVELS).astype(BF16)
            lhs_a = _factors(mixed[word_rows(t), :], _LHS)
            copies = out_copies(t)
            ready = copies[0]
            for n, y in _quadrant_sums(lambda g: _strassen(lambda i: lhs_a[i], lambda i: _wide(wo_fac, i),
                                                           levels=LEVELS - 1, base=g * PRODUCTS // 7)):
                ready.start()
                row, col = n // 2 * (ROWS // 2), n % 2 * (DM // 2)
                result[0, t & 1, row:row + ROWS // 2, col:col + DM // 2] = y.astype(BF16)
                ready = copies[1 + n]
            ready.start()

        lax.fori_loop(0, STEPS, outputs, None)
        for t in (STEPS - 2, STEPS - 1):
            for copy in out_copies(t):
                copy.wait()

    pl.run_scoped(
        attend,
        pltpu.VMEM((7 ** O_LEVELS, H * D >> O_LEVELS, DM >> O_LEVELS), BF16),
        pltpu.VMEM((4, S, D), BF16), pltpu.VMEM((2, 2, ROWS, DM), BF16))


@jax.jit
def pallas_concat_heads__sliding_local_dilated__compressed_kv_cla__prompt_kernel(
    A_x: jax.Array,
    A_wqkv: jax.Array,
    A_wo: jax.Array,
    B_x: jax.Array,
    B_c_kv: jax.Array,
    B_w_q: jax.Array,
    B_w_uk: jax.Array,
    B_w_uv: jax.Array,
    B_w_o: jax.Array,
):
    assert A_x.shape == B_x.shape == (1, S, DM) and B_c_kv.shape == (1, S, DC)
    assert B_w_q.shape == (DM, H, D) and B_w_uk.shape == B_w_uv.shape == (DC, H, D)
    out = pl.pallas_call(
        _kernel,
        out_shape=jax.ShapeDtypeStruct((S, 2 * DM), BF16),
        in_specs=[pl.BlockSpec(memory_space=pl.ANY)] * 9,
        out_specs=pl.BlockSpec(memory_space=pl.ANY),
        scratch_shapes=[
            pltpu.VMEM((2, 2, DC, D), U32), pltpu.VMEM((2, 2 ** O_LEVELS, D >> O_LEVELS, DM), U32),
            pltpu.VMEM((S // CHUNK, PRODUCTS, CHUNK // 4, DC // 4), BF16),
            pltpu.VMEM((PRODUCTS, DC // 4, D), BF16), pltpu.VMEM((PRODUCTS, DM // 512, DM // 4, 128), BF16),
            pltpu.VMEM((H, S, D), BF16), pltpu.VMEM((S // 2, DM), U32),
            pltpu.SemaphoreType.DMA((4,)), pltpu.SemaphoreType.DMA((2,)),
        ],
        compiler_params=pltpu.CompilerParams(vmem_limit_bytes=120 * 1024 * 1024),
        name="concat_heads_attention",
    )(
        A_x.reshape(S, DM), A_wqkv.reshape(4, DM // 4, 3 * DM), A_wo.reshape(4, DM // 4, DM),
        B_x.reshape(S, DM), B_c_kv.reshape(S, DC), B_w_q.reshape(4, DM // 4, H // 2, 2, D),
        B_w_uk.reshape(DC, H // 2, 2, D), B_w_uv.reshape(DC, H // 2, 2, D),
        B_w_o.reshape(2 ** O_LEVELS, H * D >> O_LEVELS, DM),
    )
    return out.reshape(1, S, 2 * DM)
```
